```python
import jax
import jax.numpy as jnp

def _softmax(x, axis=-1):
    return jax.nn.softmax(x, axis=axis)

def _gelu(x):
    return jax.nn.gelu(x, approximate=True)

def _silu(x):
    return jax.nn.silu(x)

def _sigmoid(x):
    return jax.nn.sigmoid(x)

def _layernorm(x, axis=-1, eps=1e-05):
    m = jnp.mean(x, axis=axis, keepdims=True)
    v = jnp.var(x, axis=axis, keepdims=True)
    return (x - m) / jnp.sqrt(v + eps)

def _scatter_add(tgt, idx, src, axis=0):
    return tgt.at[idx].add(src)

def _segment_sum(src, seg, n):
    return jax.ops.segment_sum(src, seg, n)

class _Rng:

    def __init__(self, key):
        self._k = key

    def _next(self):
        self._k, sub = jax.random.split(self._k)
        return sub

    def normal(self, shape):
        return jax.random.normal(self._next(), shape, dtype=jnp.bfloat16)

    def randint(self, lo, hi, shape):
        return jax.random.randint(self._next(), shape, lo, hi, dtype=jnp.int32)

    def uniform(self, shape, lo=0.0, hi=1.0):
        return jax.random.uniform(self._next(), shape, jnp.bfloat16, lo, hi)

    def permutation(self, n):
        return jax.random.permutation(self._next(), n)
kernel_name = 'interleave_layers__memory_aug_recurrent_mem_tr__mixer_s_mlp__prompt'

def setup_inputs():
    _rng = _Rng(jax.random.key(int.from_bytes(__import__("os").urandom(4), "little")))
    _w = lambda a: (lambda t: t.astype(jnp.bfloat16) if jnp.issubdtype(t.dtype, jnp.floating) else t)(jnp.asarray(a))

    def _A_setup():
        B, S, Dm = (1, 2048, 640)
        H, Dh = (32, 192)
        M, seg = (8, 32)
        seg = min(seg, S)
        S = S // seg * seg
        return {'x': _w((lambda *s: _rng.normal(s) * 0.05)(B, S, Dm)), 'mem0': _w((lambda *s: _rng.normal(s) * 0.05)(B, M, Dm)), 'Wq': _w((lambda *s: _rng.normal(s) * 0.05)(Dm, H, Dh) * Dm ** (-0.5)), 'Wk': _w((lambda *s: _rng.normal(s) * 0.05)(Dm, H, Dh) * Dm ** (-0.5)), 'Wv': _w((lambda *s: _rng.normal(s) * 0.05)(Dm, H, Dh) * Dm ** (-0.5)), 'Wo': _w((lambda *s: _rng.normal(s) * 0.05)(H, Dh, Dm) * (H * Dh) ** (-0.5)), 'seg_len': seg}
    _A_in = _A_setup()

    def _B_setup():
        B, S, D, F = (1, 2048, 640, 1536)
        return {'x': _w((lambda *s: _rng.normal(s) * 0.05)(B, S, D)), 'w1': _w((lambda *s: _rng.normal(s) * 0.05)(D, D) * D ** (-0.5)), 'w2': _w((lambda *s: _rng.normal(s) * 0.05)(D, D) * D ** (-0.5)), 'w3': _w((lambda *s: _rng.normal(s) * 0.05)(D, F) * D ** (-0.5)), 'w4': _w((lambda *s: _rng.normal(s) * 0.05)(F, D) * F ** (-0.5))}
    _B_in = _B_setup()
    return {'A_x': _A_in['x'], 'A_mem0': _A_in['mem0'], 'A_Wq': _A_in['Wq'], 'A_Wk': _A_in['Wk'], 'A_Wv': _A_in['Wv'], 'A_Wo': _A_in['Wo'], 'A_seg_len': _A_in['seg_len'], 'B_x': _B_in['x'], 'B_w1': _B_in['w1'], 'B_w2': _B_in['w2'], 'B_w3': _B_in['w3'], 'B_w4': _B_in['w4']}

def reference(A_x, A_mem0, A_Wq, A_Wk, A_Wv, A_Wo, A_seg_len, B_x, B_w1, B_w2, B_w3, B_w4):

    def _A_ref(x, mem0, Wq, Wk, Wv, Wo, seg_len):
        B, S, Dm = x.shape
        H, Dh = (Wq.shape[1], Wq.shape[2])
        M = mem0.shape[1]
        scale = Dh ** (-0.5)
        n_seg = S // seg_len
        L = M + seg_len
        idx = jnp.arange(L)
        mask = (idx[:, None] < M) | (idx[:, None] >= idx[None, :])
        mem = mem0
        outs = []
        for s in range(n_seg):
            xs = x[:, s * seg_len:(s + 1) * seg_len, :].copy()
            h = jnp.concatenate([mem, xs], axis=1)
            q = jnp.einsum('btd,dhe->bhte', h, Wq)
            k = jnp.einsum('btd,dhe->bhte', h, Wk)
            v = jnp.einsum('btd,dhe->bhte', h, Wv)
            scores = jnp.einsum('bhqe,bhke->bhqk', q, k) * scale
            scores = jnp.where(mask[None, None], scores, -1000000000.0)
            p = _softmax(scores, axis=-1)
            o = jnp.einsum('bhqk,bhke->bhqe', p, v)
            o = jnp.einsum('bhte,hed->btd', o, Wo)
            mem = o[:, :M, :].copy()
            outs.append(o[:, M:, :])
        return jnp.concatenate(outs, axis=1)

    def _B_ref(x, w1, w2, w3, w4):
        B, S, D = x.shape
        h = _gelu(_layernorm(x, axis=-1) @ w1)
        c = D // 4
        g0 = jnp.pad(h[:, :, 0 * c:1 * c], ((0, 0), (1, 0), (0, 0)))[:, :S, :]
        g1 = jnp.pad(h[:, :, 1 * c:2 * c], ((0, 0), (0, 1), (0, 0)))[:, 1:, :]
        g2 = jnp.pad(h[:, :, 2 * c:3 * c], ((0, 0), (2, 0), (0, 0)))[:, :S, :]
        g3 = jnp.pad(h[:, :, 3 * c:], ((0, 0), (0, 2), (0, 0)))[:, 2:, :]
        hs = jnp.concatenate([g0, g1, g2, g3], axis=-1) @ w2
        x1 = x + hs
        h2 = _gelu(_layernorm(x1, axis=-1) @ w3) @ w4
        return x1 + h2
    x = A_x
    x = x + _A_ref(_layernorm(x, axis=-1), A_mem0, A_Wq, A_Wk, A_Wv, A_Wo, A_seg_len)
    x = x + _B_ref(_layernorm(x, axis=-1), B_w1, B_w2, B_w3, B_w4)
    x = x + _A_ref(_layernorm(x, axis=-1), A_mem0, A_Wq, A_Wk, A_Wv, A_Wo, A_seg_len)
    x = x + _B_ref(_layernorm(x, axis=-1), B_w1, B_w2, B_w3, B_w4)
    return x
```

```python
import jax
import jax.numpy as jnp
import jax.experimental.pallas as pl
import jax.experimental.pallas.tpu as pltpu

S = 2048
D = 640
NH = 32
DH = 192
M = 8
SEG = 32
L = M + SEG
NSEG = S // SEG
F = 1536
NP = NH // 2
PW = 2 * DH
EPS = 1e-5
SCALE = DH ** -0.5
LOG2E = 1.4426950408889634
PAD = 8
TB = 256
NB = S // TB

NT = (((1,), (1,)), ((), ()))
NN = (((1,), (0,)), ((), ()))
f32 = jnp.float32
bf16 = jnp.bfloat16


def _dot(a, b, dims=NN):
    return jax.lax.dot_general(a, b, dims, preferred_element_type=f32)


def _ln(x):
    m = jnp.mean(x, axis=-1, keepdims=True)
    xc = x - m
    v = jnp.mean(xc * xc, axis=-1, keepdims=True)
    return xc * jax.lax.rsqrt(v + EPS)


def _gelu(x):
    return jax.nn.gelu(x, approximate=True)


def _w(ref_val):
    return pltpu.bitcast(ref_val, bf16)


def _blockdiag(x2, lane64):
    z = jnp.zeros((L, 128), x2.dtype)
    a, b, c = x2[:, 0:128], x2[:, 128:256], x2[:, 256:384]
    top = jnp.concatenate([a, jnp.where(lane64, b, 0.0), z], axis=1)
    bot = jnp.concatenate([z, jnp.where(lane64, 0.0, b), c], axis=1)
    return jnp.concatenate([top, bot], axis=0)


def _kernel(x_hbm, mem0_hbm, wq_hbm, wk_hbm, wv_hbm, wo_hbm,
            w1_hbm, w2_hbm, w3_hbm, w4_hbm, out_hbm,
            xb, memb, stage, wqkv, wo_s, w1_s, w2_s, w3_s, w4_s,
            X, H, Y, HB, qkv_s, o_s, ob,
            sem_x, sem_w, sem_b, sem_o):

    cp_x = pltpu.make_async_copy(x_hbm, xb, sem_x.at[0])
    cp_m = pltpu.make_async_copy(mem0_hbm, memb, sem_x.at[1])
    cp_x.start()
    cp_m.start()

    def w_copies(hp):
        r0 = hp * PW if isinstance(hp, int) else pl.multiple_of(hp * PW, 128)
        return [pltpu.make_async_copy(src.at[pl.ds(r0, PW), :],
                                      stage.at[a, pl.ds(r0, PW), :], sem_w.at[hp])
                for a, src in enumerate((wq_hbm, wk_hbm, wv_hbm))]

    for hp in range(NP):
        for c in w_copies(hp):
            c.start()
    cp_wo = pltpu.make_async_copy(wo_hbm.bitcast(jnp.int32), wo_s, sem_b.at[0])
    cp_wo.start()
    cp_b = [pltpu.make_async_copy(src.bitcast(jnp.int32), dst, sem_b.at[1 + i])
            for i, (src, dst) in enumerate(((w1_hbm, w1_s), (w2_hbm, w2_s),
                                            (w3_hbm, w3_s), (w4_hbm, w4_s)))]
    for c in cp_b:
        c.start()

    HB[0:PAD, :] = jnp.zeros((PAD, D), f32)
    HB[PAD + S:PAD + S + PAD, :] = jnp.zeros((PAD, D), f32)

    cp_x.wait()
    cp_m.wait()

    def ln0(i, _):
        r = pl.ds(pl.multiple_of(i * 128, 128), 128)
        xv = xb[r, :].astype(f32)
        X[r, :] = xv
        H[r, :] = _ln(xv)
        return 0
    jax.lax.fori_loop(0, S // 128, ln0, 0)

    def tr(hp, _):
        for c in w_copies(hp):
            c.wait()
        r0 = pl.multiple_of(hp * PW, 128)
        for a in range(3):
            for kt in range(D // 128):
                t = stage[a, pl.ds(r0, PW), kt * 128:(kt + 1) * 128].T
                wqkv[hp, kt * 64:(kt + 1) * 64, a * PW:(a + 1) * PW] = pltpu.bitcast(t, jnp.int32)
        return 0
    jax.lax.fori_loop(0, NP, tr, 0)

    cp_wo.wait()

    lane64 = jax.lax.broadcasted_iota(jnp.int32, (L, 128), 1) < 64
    ri = jax.lax.broadcasted_iota(jnp.int32, (L, 2 * L), 0)
    ci = jax.lax.broadcasted_iota(jnp.int32, (L, 2 * L), 1)
    first = ci < L
    causal = (ri < M) | (ri >= jnp.where(first, ci, ci - L))

    def a_step(s, mem):
        rows = pl.ds(pl.multiple_of(s * SEG, SEG), SEG)
        h = jnp.concatenate([mem, H[rows, :]], axis=0)
        sc, pr = {}, {}
        acc = [None]

        def st_qkv(hp):
            qkv_s[hp] = _dot(h, _w(wqkv[hp]))

        def st_qk(hp):
            sc[hp] = _dot(qkv_s[hp, :, 0:PW], _blockdiag(qkv_s[hp, :, PW:2 * PW], lane64), NT)

        def st_softmax(hp):
            v = jnp.where(causal, sc.pop(hp), -1e9 / SCALE)
            m0 = jnp.max(jnp.where(first, v, -jnp.inf), axis=1, keepdims=True)
            m1 = jnp.max(jnp.where(first, -jnp.inf, v), axis=1, keepdims=True)
            e = jnp.exp2((v - jnp.where(first, m0, m1)) * (SCALE * LOG2E))
            l0 = jnp.sum(jnp.where(first, e, 0.0), axis=1, keepdims=True)
            l1 = jnp.sum(jnp.where(first, 0.0, e), axis=1, keepdims=True)
            pr[hp] = e * jnp.where(first, 1.0 / l0, 1.0 / l1)

        def st_pv(hp):
            o_s[:, hp * PW:(hp + 1) * PW] = _dot(
                pr.pop(hp), _blockdiag(qkv_s[hp, :, 2 * PW:3 * PW], lane64))

        def st_out(hp):
            t = _dot(o_s[:, hp * PW:(hp + 1) * PW], _w(wo_s[hp * DH:(hp + 1) * DH, :]))
            acc[0] = t if acc[0] is None else acc[0] + t

        for i in range(NP + 4):
            if i < NP:
                st_qkv(i)
            if 0 <= i - 1 < NP:
                st_qk(i - 1)
            if 0 <= i - 2 < NP:
                st_softmax(i - 2)
            if 0 <= i - 3 < NP:
                st_pv(i - 3)
            if 0 <= i - 4 < NP:
                st_out(i - 4)
        X[rows, :] = X[rows, :] + acc[0][M:, :]
        return acc[0][:M, :]

    def b_phase1(i, _):
        r = pl.ds(pl.multiple_of(i * TB, TB), TB)
        y = _ln(X[r, :])
        Y[r, :] = y
        HB[pl.ds(pl.multiple_of(i * TB + PAD, PAD), TB), :] = _gelu(_dot(_ln(y), _w(w1_s[...])))
        return 0

    lane = jax.lax.broadcasted_iota(jnp.int32, (TB, 128), 1)

    def b_phase2(i, layer):
        r = pl.ds(pl.multiple_of(i * TB, TB), TB)
        win = HB[pl.ds(pl.multiple_of(i * TB, TB), TB + 2 * PAD), :]

        def sh(ct, d):
            return win[PAD + d:PAD + d + TB, ct * 128:(ct + 1) * 128]
        hs_in = jnp.concatenate([
            sh(0, -1),
            jnp.where(lane < 32, sh(1, -1), sh(1, 1)),
            jnp.where(lane < 64, sh(2, 1), sh(2, -2)),
            jnp.where(lane < 96, sh(3, -2), sh(3, 2)),
            sh(4, 2)], axis=1)
        x1 = Y[r, :] + _dot(hs_in, _w(w2_s[...]))
        g = _gelu(_dot(_ln(x1), _w(w3_s[...])))
        xn = X[r, :] + (x1 + _dot(g, _w(w4_s[...])))
        X[r, :] = xn
        H[r, :] = _ln(xn)
        ob[r, :] = xn.astype(bf16)

        @pl.when(layer == 1)
        def _():
            pltpu.make_async_copy(ob.at[r, :], out_hbm.at[r, :], sem_o.at[i]).start()
        return layer

    def layer_body(layer, _):
        jax.lax.fori_loop(0, NSEG, a_step, memb[...].astype(f32))

        @pl.when(layer == 0)
        def _():
            for c in cp_b:
                c.wait()
        jax.lax.fori_loop(0, NB, b_phase1, 0)
        jax.lax.fori_loop(0, NB, b_phase2, layer)
        return 0

    jax.lax.fori_loop(0, 2, layer_body, 0)

    for i in range(NB):
        pltpu.make_async_copy(ob.at[pl.ds(i * TB, TB), :], out_hbm.at[pl.ds(i * TB, TB), :],
                              sem_o.at[i]).wait()


def pallas_interleave_layers__memory_aug_recurrent_mem_tr__mixer_s_mlp__prompt_kernel(
    A_x: jax.Array,
    A_mem0: jax.Array,
    A_Wq: jax.Array,
    A_Wk: jax.Array,
    A_Wv: jax.Array,
    A_Wo: jax.Array,
    A_seg_len,
    B_x: jax.Array,
    B_w1: jax.Array,
    B_w2: jax.Array,
    B_w3: jax.Array,
    B_w4: jax.Array,
):
    del A_seg_len, B_x

    def wt(w):
        return jnp.transpose(w, (1, 2, 0)).reshape(NH * DH, D)

    any_spec = pl.BlockSpec(memory_space=pl.ANY)
    out = pl.pallas_call(
        _kernel,
        out_shape=jax.ShapeDtypeStruct((S, D), bf16),
        in_specs=[any_spec] * 10,
        out_specs=any_spec,
        scratch_shapes=[
            pltpu.VMEM((S, D), bf16),
            pltpu.VMEM((M, D), bf16),
            pltpu.VMEM((3, NH * DH, D), bf16),
            pltpu.VMEM((NP, D // 2, 3 * PW), jnp.int32),
            pltpu.VMEM((NH * DH // 2, D), jnp.int32),
            pltpu.VMEM((D // 2, D), jnp.int32),
            pltpu.VMEM((D // 2, D), jnp.int32),
            pltpu.VMEM((D // 2, F), jnp.int32),
            pltpu.VMEM((F // 2, D), jnp.int32),
            pltpu.VMEM((S, D), f32),
            pltpu.VMEM((S, D), f32),
            pltpu.VMEM((S, D), f32),
            pltpu.VMEM((S + 2 * PAD, D), f32),
            pltpu.VMEM((NP, L, 3 * PW), f32),
            pltpu.VMEM((L, NH * DH), f32),
            pltpu.VMEM((S, D), bf16),
            pltpu.SemaphoreType.DMA((2,)),
            pltpu.SemaphoreType.DMA((NP,)),
            pltpu.SemaphoreType.DMA((5,)),
            pltpu.SemaphoreType.DMA((NB,)),
        ],
        compiler_params=pltpu.CompilerParams(vmem_limit_bytes=120 * 1024 * 1024),
    )(A_x.reshape(S, D), A_mem0.reshape(M, D), wt(A_Wq), wt(A_Wk), wt(A_Wv),
      A_Wo.reshape(NH * DH, D), B_w1, B_w2, B_w3, B_w4)
    return out.reshape(1, S, D)
```

```python
import functools

import jax
import jax.numpy as jnp
import jax.experimental.pallas as pl
import jax.experimental.pallas.tpu as pltpu

S = 2048
D = 640
NH = 32
DH = 192
M = 8
SEG = 32
L = M + SEG
NSEG = S // SEG
F = 1536
NP = NH // 2
PW = 2 * DH
EPS = 1e-5
SCALE = DH ** -0.5
LOG2E = 1.4426950408889634
PAD = 8
TB = 256
NB = S // TB
NPRE = 40
RPRE = NPRE * M
SIN = SEG - M
NSLOT = 4

NT = (((1,), (1,)), ((), ()))
NN = (((1,), (0,)), ((), ()))
f32 = jnp.float32
bf16 = jnp.bfloat16


def _dot(a, b, dims=NN):
    return jax.lax.dot_general(a, b, dims, preferred_element_type=f32)


def _ln(x):
    m = jnp.mean(x, axis=-1, keepdims=True)
    xc = x - m
    v = jnp.mean(xc * xc, axis=-1, keepdims=True)
    return xc * jax.lax.rsqrt(v + EPS)


def _gelu(x):
    return jax.nn.gelu(x, approximate=True)


def _w(ref_val):
    return pltpu.bitcast(ref_val, bf16)


def _blockdiag(x2, lane64):
    z = jnp.zeros((L, 128), x2.dtype)
    a, b, c = x2[:, 0:128], x2[:, 128:256], x2[:, 256:384]
    top = jnp.concatenate([a, jnp.where(lane64, b, 0.0), z], axis=1)
    bot = jnp.concatenate([z, jnp.where(lane64, 0.0, b), c], axis=1)
    return jnp.concatenate([top, bot], axis=0)


def _kernel(x_hbm, mem0_hbm, wq_hbm, wk_hbm, wv_hbm, wo_hbm,
            w1_hbm, w2_hbm, w3_hbm, w4_hbm, out_hbm,
            xb, memb, stage, wqkv, wo_s, w1_s, w2_s, w3_s, w4_s,
            X, H, Y, HB, HL, PRE, qkv_s, o_s, ob,
            sem_x, sem_w, sem_b, sem_o):

    cp_x = pltpu.make_async_copy(x_hbm, xb, sem_x.at[0])
    cp_m = pltpu.make_async_copy(mem0_hbm, memb.at[0:M, :], sem_x.at[1])
    cp_x.start()
    cp_m.start()

    def w_copies(hp):
        r0 = hp * PW if isinstance(hp, int) else pl.multiple_of(hp * PW, 128)
        slot = hp % NSLOT
        return [pltpu.make_async_copy(src.at[pl.ds(r0, PW), :], stage.at[slot, a], sem_w.at[slot])
                for a, src in enumerate((wq_hbm, wk_hbm, wv_hbm))]

    for hp in range(2):
        for c in w_copies(hp):
            c.start()
    def wo_copy(hp):
        r0 = hp * DH if isinstance(hp, int) else pl.multiple_of(hp * DH, 64)
        return pltpu.make_async_copy(wo_hbm.bitcast(jnp.int32).at[pl.ds(r0, DH), :],
                                     wo_s.at[pl.ds(r0, DH), :], sem_b.at[0])
    cp_b = [pltpu.make_async_copy(src.bitcast(jnp.int32), dst, sem_b.at[1 + i])
            for i, (src, dst) in enumerate(((w1_hbm, w1_s), (w2_hbm, w2_s),
                                            (w3_hbm, w3_s), (w4_hbm, w4_s)))]

    HB[0:PAD, :] = jnp.zeros((PAD, D), f32)
    HB[PAD + S:PAD + S + PAD, :] = jnp.zeros((PAD, D), f32)

    cp_x.wait()
    cp_m.wait()

    def ln0(i, _):
        r = pl.ds(pl.multiple_of(i * 128, 128), 128)
        X[r, :] = xb[r, :].astype(f32)
        return 0
    jax.lax.fori_loop(0, S // 128, ln0, 0)

    def ln_left(i, _):
        xs = [X[pl.ds(pl.multiple_of((i * 16 + j) * SEG + SIN, M), M), :] for j in range(16)]
        HL[pl.ds(pl.multiple_of(i * 128, 128), 128), :] = _ln(jnp.concatenate(xs, axis=0))
        return 0
    jax.lax.fori_loop(0, RPRE // 128, ln_left, 0)
    if RPRE % 128:
        i = RPRE // 128
        n = (RPRE % 128) // M
        xs = [X[pl.ds((i * 16 + j) * SEG + SIN, M), :] for j in range(n)]
        HL[pl.ds(i * 128, n * M), :] = _ln(jnp.concatenate(xs, axis=0))

    def tr(hp, _):
        for c in w_copies(hp):
            c.wait()

        @pl.when(hp + 2 < NP)
        def _():
            for c in w_copies(hp + 2):
                c.start()

        wo_copy(hp).start()
        slot = hp % NSLOT
        for a in range(3):
            PRE[hp, :, a * PW:(a + 1) * PW] = _dot(HL[...], stage[slot, a], NT)
            for kt in range(D // 128):
                t = stage[slot, a, :, kt * 128:(kt + 1) * 128].T
                wqkv[hp, kt * 64:(kt + 1) * 64, a * PW:(a + 1) * PW] = pltpu.bitcast(t, jnp.int32)
        return 0
    jax.lax.fori_loop(0, NP, tr, 0)

    for hp in range(NP):
        wo_copy(hp).wait()
    for c in cp_b:
        c.start()

    lane64 = jax.lax.broadcasted_iota(jnp.int32, (L, 128), 1) < 64
    ri = jax.lax.broadcasted_iota(jnp.int32, (L, 2 * L), 0)
    ci = jax.lax.broadcasted_iota(jnp.int32, (L, 2 * L), 1)
    first = ci < L
    causal = (ri < M) | (ri >= jnp.where(first, ci, ci - L))

    def a_step(s, mem, pre):
        rows = pl.ds(pl.multiple_of(s * SEG, SEG), SEG)
        nin = SIN if pre else SEG
        h = jnp.concatenate([mem, H[pl.ds(pl.multiple_of(s * SEG, SEG), nin), :]], axis=0)
        nrows = pl.ds(pl.multiple_of(jnp.minimum(s + 1, NSEG - 1) * SEG, SEG), SEG)
        H[nrows, :] = _ln(X[nrows, :])
        sc, pr = {}, {}
        acc = [None]

        def st_qkv(hp):
            qkv_s[hp, 0:M + nin, :] = _dot(h, _w(wqkv[hp]))

        def part(hp, a):
            v = qkv_s[hp, 0:M + nin, a * PW:(a + 1) * PW]
            if pre:
                v = jnp.concatenate(
                    [v, PRE[hp, pl.ds(pl.multiple_of(s * M, M), M), a * PW:(a + 1) * PW]], axis=0)
            return v

        def st_qk(hp):
            sc[hp] = _dot(part(hp, 0), _blockdiag(part(hp, 1), lane64), NT)

        def st_softmax(hp):
            v = jnp.where(causal, sc.pop(hp), -1e9 / SCALE)
            m0 = jnp.max(jnp.where(first, v, -jnp.inf), axis=1, keepdims=True)
            m1 = jnp.max(jnp.where(first, -jnp.inf, v), axis=1, keepdims=True)
            e = jnp.exp2((v - jnp.where(first, m0, m1)) * (SCALE * LOG2E))
            l0 = jnp.sum(jnp.where(first, e, 0.0), axis=1, keepdims=True)
            l1 = jnp.sum(jnp.where(first, 0.0, e), axis=1, keepdims=True)
            pr[hp] = e * jnp.where(first, 1.0 / l0, 1.0 / l1)

        def st_pv(hp):
            o_s[:, hp * PW:(hp + 1) * PW] = _dot(pr.pop(hp), _blockdiag(part(hp, 2), lane64))

        def st_out(hp):
            t = _dot(o_s[:, hp * PW:(hp + 1) * PW], _w(wo_s[hp * DH:(hp + 1) * DH, :]))
            acc[0] = t if acc[0] is None else acc[0] + t

        for i in range(NP + 4):
            if i < NP:
                st_qkv(i)
            if 0 <= i - 1 < NP:
                st_qk(i - 1)
            if 0 <= i - 2 < NP:
                st_softmax(i - 2)
            if 0 <= i - 3 < NP:
                st_pv(i - 3)
            if 0 <= i - 4 < NP:
                st_out(i - 4)
        X[rows, :] = X[rows, :] + acc[0][M:, :]
        return acc[0][:M, :]

    def b_phase1(i, _):
        r = pl.ds(pl.multiple_of(i * TB, TB), TB)
        y = _ln(X[r, :])
        Y[r, :] = y
        HB[pl.ds(pl.multiple_of(i * TB + PAD, PAD), TB), :] = _gelu(_dot(_ln(y), _w(w1_s[...])))
        return 0

    lane = jax.lax.broadcasted_iota(jnp.int32, (TB, 128), 1)

    def b_phase2(i, layer):
        r = pl.ds(pl.multiple_of(i * TB, TB), TB)
        win = HB[pl.ds(pl.multiple_of(i * TB, TB), TB + 2 * PAD), :]

        def sh(ct, d):
            return win[PAD + d:PAD + d + TB, ct * 128:(ct + 1) * 128]
        hs_in = jnp.concatenate([
            sh(0, -1),
            jnp.where(lane < 32, sh(1, -1), sh(1, 1)),
            jnp.where(lane < 64, sh(2, 1), sh(2, -2)),
            jnp.where(lane < 96, sh(3, -2), sh(3, 2)),
            sh(4, 2)], axis=1)
        x1 = Y[r, :] + _dot(hs_in, _w(w2_s[...]))
        g = _gelu(_dot(_ln(x1), _w(w3_s[...])))
        xn = X[r, :] + (x1 + _dot(g, _w(w4_s[...])))
        X[r, :] = xn
        ob[r, :] = xn.astype(bf16)

        @pl.when(layer == 1)
        def _():
            pltpu.make_async_copy(ob.at[r, :], out_hbm.at[r, :], sem_o.at[i]).start()
        return layer

    def layer_body(layer, _):
        H[0:SEG, :] = _ln(X[0:SEG, :])
        npre = jnp.where(layer == 0, NPRE, 0)
        mem = jax.lax.fori_loop(0, npre, functools.partial(a_step, pre=True), memb[0:M, :].astype(f32))
        jax.lax.fori_loop(npre, NSEG, functools.partial(a_step, pre=False), mem)

        @pl.when(layer == 0)
        def _():
            for c in cp_b:
                c.wait()
        jax.lax.fori_loop(0, NB, b_phase1, 0)
        jax.lax.fori_loop(0, NB, b_phase2, layer)
        return 0

    jax.lax.fori_loop(0, 2, layer_body, 0)

    for i in range(NB):
        pltpu.make_async_copy(ob.at[pl.ds(i * TB, TB), :], out_hbm.at[pl.ds(i * TB, TB), :],
                              sem_o.at[i]).wait()


def pallas_interleave_layers__memory_aug_recurrent_mem_tr__mixer_s_mlp__prompt_kernel(
    A_x: jax.Array,
    A_mem0: jax.Array,
    A_Wq: jax.Array,
    A_Wk: jax.Array,
    A_Wv: jax.Array,
    A_Wo: jax.Array,
    A_seg_len,
    B_x: jax.Array,
    B_w1: jax.Array,
    B_w2: jax.Array,
    B_w3: jax.Array,
    B_w4: jax.Array,
):
    del A_seg_len, B_x

    def wt(w):
        return jnp.transpose(w, (1, 2, 0)).reshape(NH * DH, D)

    any_spec = pl.BlockSpec(memory_space=pl.ANY)
    out = pl.pallas_call(
        _kernel,
        out_shape=jax.ShapeDtypeStruct((S, D), bf16),
        in_specs=[any_spec] * 10,
        out_specs=any_spec,
        scratch_shapes=[
            pltpu.VMEM((S, D), bf16),
            pltpu.VMEM((64, D), bf16),
            pltpu.VMEM((NSLOT, 3, PW, D), bf16),
            pltpu.VMEM((NP, D // 2, 3 * PW), jnp.int32),
            pltpu.VMEM((NH * DH // 2, D), jnp.int32),
            pltpu.VMEM((D // 2, D), jnp.int32),
            pltpu.VMEM((D // 2, D), jnp.int32),
            pltpu.VMEM((D // 2, F), jnp.int32),
            pltpu.VMEM((F // 2, D), jnp.int32),
            pltpu.VMEM((S, D), f32),
            pltpu.VMEM((S, D), f32),
            pltpu.VMEM((S, D), f32),
            pltpu.VMEM((S + 32, D), f32),
            pltpu.VMEM((RPRE, D), f32),
            pltpu.VMEM((NP, RPRE, 3 * PW), f32),
            pltpu.VMEM((NP, L, 3 * PW), f32),
            pltpu.VMEM((L, NH * DH), f32),
            pltpu.VMEM((S, D), bf16),
            pltpu.SemaphoreType.DMA((2,)),
            pltpu.SemaphoreType.DMA((NSLOT,)),
            pltpu.SemaphoreType.DMA((5,)),
            pltpu.SemaphoreType.DMA((NB,)),
        ],
        compiler_params=pltpu.CompilerParams(vmem_limit_bytes=120 * 1024 * 1024),
    )(A_x.reshape(S, D), A_mem0.reshape(M, D), wt(A_Wq), wt(A_Wk), wt(A_Wv),
      A_Wo.reshape(NH * DH, D), B_w1, B_w2, B_w3, B_w4)
    return out.reshape(1, S, D)
```

```python
import functools

import jax
import jax.numpy as jnp
import jax.experimental.pallas as pl
import jax.experimental.pallas.tpu as pltpu

S = 2048
D = 640
NH = 32
DH = 192
M = 8
SEG = 32
L = M + SEG
NSEG = S // SEG
F = 1536
NP = NH // 2
PW = 2 * DH
EPS = 1e-5
SCALE = DH ** -0.5
LOG2E = 1.4426950408889634
PAD = 8
TB = 256
NB = S // TB
NH_B = 4
NPRE = 40
RPRE = NPRE * M
SIN = SEG - M
B1_ACT_AT = 2
B1_NORM_AT = 8
B1_DOT_AT = 17
LAG_OUT = 4
UNR = 2
NSLOT = 4

NT = (((1,), (1,)), ((), ()))
NN = (((1,), (0,)), ((), ()))
f32 = jnp.float32
bf16 = jnp.bfloat16


def _dot(a, b, dims=NN):
    return jax.lax.dot_general(a, b, dims, preferred_element_type=f32)


def _ln(x):
    m = jnp.mean(x, axis=-1, keepdims=True)
    xc = x - m
    v = jnp.mean(xc * xc, axis=-1, keepdims=True)
    return xc * jax.lax.rsqrt(v + EPS)


def _gelu(x):
    return jax.nn.gelu(x, approximate=True)


def _w(ref_val):
    return pltpu.bitcast(ref_val, bf16)


def _blockdiag(x2, lane64):
    z = jnp.zeros((L, 128), x2.dtype)
    a, b, c = x2[:, 0:128], x2[:, 128:256], x2[:, 256:384]
    top = jnp.concatenate([a, jnp.where(lane64, b, 0.0), z], axis=1)
    bot = jnp.concatenate([z, jnp.where(lane64, 0.0, b), c], axis=1)
    return jnp.concatenate([top, bot], axis=0)


def _kernel(x_hbm, mem0_hbm, wq_hbm, wk_hbm, wv_hbm, wo_hbm,
            w1_hbm, w2_hbm, w3_hbm, w4_hbm, out_hbm,
            xb, memb, stage, wqkv, wo_s, w1_s, w2_s, w3_s, w4_s,
            X, H, Y, HB, HL, PRE, qkv_s, o_s, Z, PA, ob,
            sem_x, sem_w, sem_b, sem_o):

    cp_x = pltpu.make_async_copy(x_hbm, xb, sem_x.at[0])
    cp_m = pltpu.make_async_copy(mem0_hbm, memb.at[0:M, :], sem_x.at[1])
    cp_x.start()
    cp_m.start()

    def w_copies(hp):
        r0 = hp * PW if isinstance(hp, int) else pl.multiple_of(hp * PW, 128)
        slot = hp % NSLOT
        return [pltpu.make_async_copy(src.at[pl.ds(r0, PW), :], stage.at[slot, a], sem_w.at[slot])
                for a, src in enumerate((wq_hbm, wk_hbm, wv_hbm))]

    for hp in range(2):
        for c in w_copies(hp):
            c.start()
    def wo_copy(hp):
        r0 = hp * DH if isinstance(hp, int) else pl.multiple_of(hp * DH, 64)
        return pltpu.make_async_copy(wo_hbm.bitcast(jnp.int32).at[pl.ds(r0, DH), :],
                                     wo_s.at[pl.ds(r0, DH), :], sem_b.at[0])
    cp_b = [pltpu.make_async_copy(src.bitcast(jnp.int32), dst, sem_b.at[1 + i])
            for i, (src, dst) in enumerate(((w1_hbm, w1_s), (w2_hbm, w2_s),
                                            (w3_hbm, w3_s), (w4_hbm, w4_s)))]

    HB[0:PAD, :] = jnp.zeros((PAD, D), f32)
    HB[PAD + S:PAD + S + PAD, :] = jnp.zeros((PAD, D), f32)

    cp_x.wait()
    cp_m.wait()

    def ln0(i, _):
        r = pl.ds(pl.multiple_of(i * 128, 128), 128)
        X[r, :] = xb[r, :].astype(f32)
        return 0
    jax.lax.fori_loop(0, S // 128, ln0, 0)

    def ln_left(i, _):
        xs = [X[pl.ds(pl.multiple_of((i * 16 + j) * SEG + SIN, M), M), :] for j in range(16)]
        HL[pl.ds(pl.multiple_of(i * 128, 128), 128), :] = _ln(jnp.concatenate(xs, axis=0))
        return 0
    jax.lax.fori_loop(0, RPRE // 128, ln_left, 0)
    if RPRE % 128:
        i = RPRE // 128
        n = (RPRE % 128) // M
        xs = [X[pl.ds((i * 16 + j) * SEG + SIN, M), :] for j in range(n)]
        HL[pl.ds(i * 128, n * M), :] = _ln(jnp.concatenate(xs, axis=0))

    def tr(hp, _):
        for c in w_copies(hp):
            c.wait()

        @pl.when(hp + 2 < NP)
        def _():
            for c in w_copies(hp + 2):
                c.start()

        wo_copy(hp).start()

        @pl.when(hp == NP - 1)
        def _():
            cp_b[0].start()
        slot = hp % NSLOT
        for a in range(3):
            PRE[hp, :, a * PW:(a + 1) * PW] = _dot(HL[...], stage[slot, a], NT)
            for kt in range(D // 128):
                t = stage[slot, a, :, kt * 128:(kt + 1) * 128].T
                wqkv[hp, kt * 64:(kt + 1) * 64, a * PW:(a + 1) * PW] = pltpu.bitcast(t, jnp.int32)
        return 0
    jax.lax.fori_loop(0, NP, tr, 0)

    PA[...] = jnp.zeros((SEG, D), f32)
    for hp in range(NP):
        wo_copy(hp).wait()
    cp_b[0].wait()
    for c in cp_b[1:]:
        c.start()

    lane64 = jax.lax.broadcasted_iota(jnp.int32, (L, 128), 1) < 64
    ri = jax.lax.broadcasted_iota(jnp.int32, (L, 2 * L), 0)
    ci = jax.lax.broadcasted_iota(jnp.int32, (L, 2 * L), 1)
    first = ci < L
    causal = (ri < M) | (ri >= jnp.where(first, ci, ci - L))

    def seg_rows(s, off=0):
        return pl.ds(pl.multiple_of(s * SEG + off, M), SEG)

    def b1_norm(s):
        y = _ln(X[seg_rows(s), :])
        Y[seg_rows(s), :] = y
        Z[...] = _ln(y)

    def b1_dot():
        PA[...] = _dot(Z[...], _w(w1_s[...]))

    def b1_act(s):
        HB[seg_rows(s, PAD), :] = _gelu(PA[...])

    def a_step(s, mem, pre):
        rows = pl.ds(pl.multiple_of(s * SEG, SEG), SEG)
        nin = SIN if pre else SEG
        h = jnp.concatenate([mem, H[pl.ds(pl.multiple_of(s * SEG, SEG), nin), :]], axis=0)
        nrows = pl.ds(pl.multiple_of(jnp.minimum(s + 1, NSEG - 1) * SEG, SEG), SEG)
        H[nrows, :] = _ln(X[nrows, :])
        sc, pr = {}, {}
        acc = [None]

        def st_qkv(hp):
            qkv_s[hp, 0:M + nin, :] = _dot(h, _w(wqkv[hp]))

        def part(hp, a):
            v = qkv_s[hp, 0:M + nin, a * PW:(a + 1) * PW]
            if pre:
                v = jnp.concatenate(
                    [v, PRE[hp, pl.ds(pl.multiple_of(s * M, M), M), a * PW:(a + 1) * PW]], axis=0)
            return v

        def st_qk(hp):
            sc[hp] = _dot(part(hp, 0), _blockdiag(part(hp, 1), lane64), NT)

        def st_softmax(hp):
            v = jnp.where(causal, sc.pop(hp), -1e9 / SCALE)
            m0 = jnp.max(jnp.where(first, v, -jnp.inf), axis=1, keepdims=True)
            m1 = jnp.max(jnp.where(first, -jnp.inf, v), axis=1, keepdims=True)
            e = jnp.exp2((v - jnp.where(first, m0, m1)) * (SCALE * LOG2E))
            l0 = jnp.sum(jnp.where(first, e, 0.0), axis=1, keepdims=True)
            l1 = jnp.sum(jnp.where(first, 0.0, e), axis=1, keepdims=True)
            pr[hp] = e * jnp.where(first, 1.0 / l0, 1.0 / l1)

        def st_pv(hp):
            o_s[:, hp * PW:(hp + 1) * PW] = _dot(pr.pop(hp), _blockdiag(part(hp, 2), lane64))

        def st_out(hp):
            t = _dot(o_s[:, hp * PW:(hp + 1) * PW], _w(wo_s[hp * DH:(hp + 1) * DH, :]))
            acc[0] = t if acc[0] is None else acc[0] + t

        for i in range(NP + LAG_OUT):
            if i < NP:
                st_qkv(i)
            if i == B1_ACT_AT:
                b1_act(jnp.maximum(s - 2, 0))
            if i == B1_NORM_AT:
                b1_norm(jnp.maximum(s - 1, 0))
            if i == B1_DOT_AT:
                b1_dot()
            if 0 <= i - 1 < NP:
                st_qk(i - 1)
            if 0 <= i - 2 < NP:
                st_softmax(i - 2)
            if 0 <= i - 3 < NP:
                st_pv(i - 3)
            if 0 <= i - LAG_OUT < NP:
                st_out(i - LAG_OUT)
        X[rows, :] = X[rows, :] + acc[0][M:, :]
        return acc[0][:M, :]

    TH = TB // NH_B
    lane = jax.lax.broadcasted_iota(jnp.int32, (TH, 128), 1)

    def b_phase2(i, layer):
        r = pl.ds(pl.multiple_of(i * TB, TB), TB)
        rows = [pl.ds(pl.multiple_of(i * TB + u * TH, TH), TH) for u in range(NH_B)]

        def mixed(u):
            win = HB[pl.ds(pl.multiple_of(i * TB + u * TH, TH), TH + 2 * PAD), :]

            def sh(ct, d):
                return win[PAD + d:PAD + d + TH, ct * 128:(ct + 1) * 128]
            return jnp.concatenate([
                sh(0, -1),
                jnp.where(lane < 32, sh(1, -1), sh(1, 1)),
                jnp.where(lane < 64, sh(2, 1), sh(2, -2)),
                jnp.where(lane < 96, sh(3, -2), sh(3, 2)),
                sh(4, 2)], axis=1)

        x1 = [Y[rows[u], :] + _dot(mixed(u), _w(w2_s[...])) for u in range(NH_B)]
        g = [_gelu(_dot(_ln(x1[u]), _w(w3_s[...]))) for u in range(NH_B)]
        for u in range(NH_B):
            xn = X[rows[u], :] + (x1[u] + _dot(g[u], _w(w4_s[...])))
            X[rows[u], :] = xn
            ob[rows[u], :] = xn.astype(bf16)

        @pl.when(layer == 1)
        def _():
            pltpu.make_async_copy(ob.at[r, :], out_hbm.at[r, :], sem_o.at[i]).start()
        return layer

    def layer_body(layer, _):
        H[0:SEG, :] = _ln(X[0:SEG, :])
        def a_steps(j, mem, pre):
            for u in range(UNR):
                mem = a_step(j * UNR + u, mem, pre)
            return mem
        npre = jnp.where(layer == 0, NPRE // UNR, 0)
        mem = jax.lax.fori_loop(0, npre, functools.partial(a_steps, pre=True), memb[0:M, :].astype(f32))
        jax.lax.fori_loop(npre, NSEG // UNR, functools.partial(a_steps, pre=False), mem)

        @pl.when(layer == 0)
        def _():
            for c in cp_b[1:]:
                c.wait()
        b1_act(NSEG - 2)
        b1_norm(NSEG - 1)
        b1_dot()
        b1_act(NSEG - 1)
        jax.lax.fori_loop(0, NB, b_phase2, layer)
        return 0

    jax.lax.fori_loop(0, 2, layer_body, 0)

    for i in range(NB):
        pltpu.make_async_copy(ob.at[pl.ds(i * TB, TB), :], out_hbm.at[pl.ds(i * TB, TB), :],
                              sem_o.at[i]).wait()


def pallas_interleave_layers__memory_aug_recurrent_mem_tr__mixer_s_mlp__prompt_kernel(
    A_x: jax.Array,
    A_mem0: jax.Array,
    A_Wq: jax.Array,
    A_Wk: jax.Array,
    A_Wv: jax.Array,
    A_Wo: jax.Array,
    A_seg_len,
    B_x: jax.Array,
    B_w1: jax.Array,
    B_w2: jax.Array,
    B_w3: jax.Array,
    B_w4: jax.Array,
):
    del A_seg_len, B_x

    def wt(w):
        return jnp.transpose(w, (1, 2, 0)).reshape(NH * DH, D)

    any_spec = pl.BlockSpec(memory_space=pl.ANY)
    out = pl.pallas_call(
        _kernel,
        out_shape=jax.ShapeDtypeStruct((S, D), bf16),
        in_specs=[any_spec] * 10,
        out_specs=any_spec,
        scratch_shapes=[
            pltpu.VMEM((S, D), bf16),
            pltpu.VMEM((64, D), bf16),
            pltpu.VMEM((NSLOT, 3, PW, D), bf16),
            pltpu.VMEM((NP, D // 2, 3 * PW), jnp.int32),
            pltpu.VMEM((NH * DH // 2, D), jnp.int32),
            pltpu.VMEM((D // 2, D), jnp.int32),
            pltpu.VMEM((D // 2, D), jnp.int32),
            pltpu.VMEM((D // 2, F), jnp.int32),
            pltpu.VMEM((F // 2, D), jnp.int32),
            pltpu.VMEM((S, D), f32),
            pltpu.VMEM((S, D), f32),
            pltpu.VMEM((S, D), f32),
            pltpu.VMEM((S + 32, D), f32),
            pltpu.VMEM((RPRE, D), f32),
            pltpu.VMEM((NP, RPRE, 3 * PW), f32),
            pltpu.VMEM((NP, L, 3 * PW), f32),
            pltpu.VMEM((L, NH * DH), f32),
            pltpu.VMEM((SEG, D), f32),
            pltpu.VMEM((SEG, D), f32),
            pltpu.VMEM((S, D), bf16),
            pltpu.SemaphoreType.DMA((2,)),
            pltpu.SemaphoreType.DMA((NSLOT,)),
            pltpu.SemaphoreType.DMA((5,)),
            pltpu.SemaphoreType.DMA((NB,)),
        ],
        compiler_params=pltpu.CompilerParams(vmem_limit_bytes=120 * 1024 * 1024),
    )(A_x.reshape(S, D), A_mem0.reshape(M, D), wt(A_Wq), wt(A_Wk), wt(A_Wv),
      A_Wo.reshape(NH * DH, D), B_w1, B_w2, B_w3, B_w4)
    return out.reshape(1, S, D)
```

```python
import functools

import jax
import jax.numpy as jnp
import jax.experimental.pallas as pl
import jax.experimental.pallas.tpu as pltpu

S = 2048
D = 640
NH = 32
DH = 192
M = 8
SEG = 32
L = M + SEG
NSEG = S // SEG
F = 1536
NP = NH // 2
PW = 2 * DH
EPS = 1e-5
SCALE = DH ** -0.5
LOG2E = 1.4426950408889634
PAD = 8
TB = 256
NB = S // TB
NH_B = 4
NPRE = 40
RPRE = NPRE * M
SIN = SEG - M
B1_ACT_AT = 2
B1_NORM_AT = 8
B1_DOT_AT = 17
LAG_OUT = 4
UNR = 2
NSLOT = 4

NT = (((1,), (1,)), ((), ()))
NN = (((1,), (0,)), ((), ()))
f32 = jnp.float32
bf16 = jnp.bfloat16


def _dot(a, b, dims=NN):
    return jax.lax.dot_general(a, b, dims, preferred_element_type=f32)


def _ln(x):
    m = jnp.mean(x, axis=-1, keepdims=True)
    xc = x - m
    v = jnp.mean(xc * xc, axis=-1, keepdims=True)
    return xc * jax.lax.rsqrt(v + EPS)


def _gelu(x):
    return jax.nn.gelu(x, approximate=True)


def _w(ref_val):
    return pltpu.bitcast(ref_val, bf16)


def _blockdiag(x2, lane64):
    z = jnp.zeros((L, 128), x2.dtype)
    a, b, c = x2[:, 0:128], x2[:, 128:256], x2[:, 256:384]
    top = jnp.concatenate([a, jnp.where(lane64, b, 0.0), z], axis=1)
    bot = jnp.concatenate([z, jnp.where(lane64, 0.0, b), c], axis=1)
    return jnp.concatenate([top, bot], axis=0)


def _kernel(x_hbm, mem0_hbm, wq_hbm, wk_hbm, wv_hbm, wo_hbm,
            w1_hbm, w2_hbm, w3_hbm, w4_hbm, out_hbm,
            xb, xl, memb, stage, wqkv, wo_s, w1_s, w2_s, w3_s, w4_s,
            X, H, Y, HB, HL, PRE, qkv_s, o_s, Z, PA, ob,
            sem_x, sem_w, sem_b, sem_o):

    cp_l = pltpu.make_async_copy(x_hbm.at[pl.ds(0, NPRE), pl.ds(SIN, M), :], xl, sem_x.at[0])
    cp_m = pltpu.make_async_copy(mem0_hbm, memb.at[0:M, :], sem_x.at[1])
    cp_l.start()

    XS = NSEG // NP

    def w_copies(hp):
        if isinstance(hp, int):
            r0, s0 = hp * PW, hp * XS
        else:
            r0, s0 = pl.multiple_of(hp * PW, 128), hp * XS
        slot = hp % NSLOT
        cps = [pltpu.make_async_copy(src.at[pl.ds(r0, PW), :], stage.at[slot, a], sem_w.at[slot])
               for a, src in enumerate((wq_hbm, wk_hbm, wv_hbm))]
        cps.append(pltpu.make_async_copy(x_hbm.at[pl.ds(s0, XS)], xb.at[pl.ds(s0, XS)],
                                         sem_w.at[slot]))
        return cps

    for hp in range(2):
        for c in w_copies(hp):
            c.start()
    cp_m.start()

    def wo_copy(hp):
        r0 = hp * DH if isinstance(hp, int) else pl.multiple_of(hp * DH, 64)
        return pltpu.make_async_copy(wo_hbm.bitcast(jnp.int32).at[pl.ds(r0, DH), :],
                                     wo_s.at[pl.ds(r0, DH), :], sem_b.at[0])
    cp_b = [pltpu.make_async_copy(src.bitcast(jnp.int32), dst, sem_b.at[1 + i])
            for i, (src, dst) in enumerate(((w1_hbm, w1_s), (w2_hbm, w2_s),
                                            (w3_hbm, w3_s), (w4_hbm, w4_s)))]

    HB[0:PAD, :] = jnp.zeros((PAD, D), f32)
    HB[PAD + S:PAD + S + PAD, :] = jnp.zeros((PAD, D), f32)
    PA[...] = jnp.zeros((SEG, D), f32)

    cp_l.wait()
    HL[...] = _ln(xl[...].astype(f32).reshape(RPRE, D))

    def tr(hp, _):
        for c in w_copies(hp):
            c.wait()

        @pl.when(hp + 2 < NP)
        def _():
            for c in w_copies(hp + 2):
                c.start()

        wo_copy(hp).start()

        @pl.when(hp == NP - 1)
        def _():
            cp_b[0].start()
        slot = hp % NSLOT
        for a in range(3):
            PRE[hp, :, a * PW:(a + 1) * PW] = _dot(HL[...], stage[slot, a], NT)
            for kt in range(D // 128):
                t = stage[slot, a, :, kt * 128:(kt + 1) * 128].T
                wqkv[hp, kt * 64:(kt + 1) * 64, a * PW:(a + 1) * PW] = pltpu.bitcast(t, jnp.int32)
        X[pl.ds(pl.multiple_of(hp * XS * SEG, XS * SEG), XS * SEG), :] = (
            xb[pl.ds(hp * XS, XS)].astype(f32).reshape(XS * SEG, D))
        return 0
    jax.lax.fori_loop(0, NP, tr, 0)

    cp_m.wait()
    for hp in range(NP):
        wo_copy(hp).wait()
    cp_b[0].wait()
    for c in cp_b[1:]:
        c.start()

    lane64 = jax.lax.broadcasted_iota(jnp.int32, (L, 128), 1) < 64
    ri = jax.lax.broadcasted_iota(jnp.int32, (L, 2 * L), 0)
    ci = jax.lax.broadcasted_iota(jnp.int32, (L, 2 * L), 1)
    first = ci < L
    causal = (ri < M) | (ri >= jnp.where(first, ci, ci - L))

    def seg_rows(s, off=0):
        return pl.ds(pl.multiple_of(s * SEG + off, M), SEG)

    def b1_norm(s):
        y = _ln(X[seg_rows(s), :])
        Y[seg_rows(s), :] = y
        Z[...] = _ln(y)

    def b1_dot():
        PA[...] = _dot(Z[...], _w(w1_s[...]))

    def b1_act(s):
        HB[seg_rows(s, PAD), :] = _gelu(PA[...])

    def a_step(s, mem, pre):
        rows = pl.ds(pl.multiple_of(s * SEG, SEG), SEG)
        nin = SIN if pre else SEG
        h = jnp.concatenate([mem, H[pl.ds(pl.multiple_of(s * SEG, SEG), nin), :]], axis=0)
        nrows = pl.ds(pl.multiple_of(jnp.minimum(s + 1, NSEG - 1) * SEG, SEG), SEG)
        H[nrows, :] = _ln(X[nrows, :])
        sc, pr = {}, {}
        acc = [None]

        def st_qkv(hp):
            qkv_s[hp, 0:M + nin, :] = _dot(h, _w(wqkv[hp]))

        def part(hp, a):
            v = qkv_s[hp, 0:M + nin, a * PW:(a + 1) * PW]
            if pre:
                v = jnp.concatenate(
                    [v, PRE[hp, pl.ds(pl.multiple_of(s * M, M), M), a * PW:(a + 1) * PW]], axis=0)
            return v

        def st_qk(hp):
            sc[hp] = _dot(part(hp, 0), _blockdiag(part(hp, 1), lane64), NT)

        def st_softmax(hp):
            v = jnp.where(causal, sc.pop(hp), -1e9 / SCALE)
            m0 = jnp.max(jnp.where(first, v, -jnp.inf), axis=1, keepdims=True)
            m1 = jnp.max(jnp.where(first, -jnp.inf, v), axis=1, keepdims=True)
            e = jnp.exp2((v - jnp.where(first, m0, m1)) * (SCALE * LOG2E))
            l0 = jnp.sum(jnp.where(first, e, 0.0), axis=1, keepdims=True)
            l1 = jnp.sum(jnp.where(first, 0.0, e), axis=1, keepdims=True)
            pr[hp] = e * jnp.where(first, 1.0 / l0, 1.0 / l1)

        def st_pv(hp):
            o_s[:, hp * PW:(hp + 1) * PW] = _dot(pr.pop(hp), _blockdiag(part(hp, 2), lane64))

        def st_out(hp):
            t = _dot(o_s[:, hp * PW:(hp + 1) * PW], _w(wo_s[hp * DH:(hp + 1) * DH, :]))
            acc[0] = t if acc[0] is None else acc[0] + t

        for i in range(NP + LAG_OUT):
            if i < NP:
                st_qkv(i)
            if i == B1_ACT_AT:
                b1_act(jnp.maximum(s - 2, 0))
            if i == B1_NORM_AT:
                b1_norm(jnp.maximum(s - 1, 0))
            if i == B1_DOT_AT:
                b1_dot()
            if 0 <= i - 1 < NP:
                st_qk(i - 1)
            if 0 <= i - 2 < NP:
                st_softmax(i - 2)
            if 0 <= i - 3 < NP:
                st_pv(i - 3)
            if 0 <= i - LAG_OUT < NP:
                st_out(i - LAG_OUT)
        X[rows, :] = X[rows, :] + acc[0][M:, :]
        return acc[0][:M, :]

    TH = TB // NH_B
    lane = jax.lax.broadcasted_iota(jnp.int32, (TH, 128), 1)

    def b_phase2(i, layer):
        r = pl.ds(pl.multiple_of(i * TB, TB), TB)
        rows = [pl.ds(pl.multiple_of(i * TB + u * TH, TH), TH) for u in range(NH_B)]

        def mixed(u):
            win = HB[pl.ds(pl.multiple_of(i * TB + u * TH, TH), TH + 2 * PAD), :]

            def sh(ct, d):
                return win[PAD + d:PAD + d + TH, ct * 128:(ct + 1) * 128]
            return jnp.concatenate([
                sh(0, -1),
                jnp.where(lane < 32, sh(1, -1), sh(1, 1)),
                jnp.where(lane < 64, sh(2, 1), sh(2, -2)),
                jnp.where(lane < 96, sh(3, -2), sh(3, 2)),
                sh(4, 2)], axis=1)

        x1 = [Y[rows[u], :] + _dot(mixed(u), _w(w2_s[...])) for u in range(NH_B)]
        g = [_gelu(_dot(_ln(x1[u]), _w(w3_s[...]))) for u in range(NH_B)]
        for u in range(NH_B):
            xn = X[rows[u], :] + (x1[u] + _dot(g[u], _w(w4_s[...])))
            X[rows[u], :] = xn
            ob[rows[u], :] = xn.astype(bf16)

        @pl.when(layer == 1)
        def _():
            pltpu.make_async_copy(ob.at[r, :], out_hbm.at[r, :], sem_o.at[i]).start()
        return layer

    def layer_body(layer, _):
        H[0:SEG, :] = _ln(X[0:SEG, :])
        def a_steps(j, mem, pre):
            for u in range(UNR):
                mem = a_step(j * UNR + u, mem, pre)
            return mem
        npre = jnp.where(layer == 0, NPRE // UNR, 0)
        mem = jax.lax.fori_loop(0, npre, functools.partial(a_steps, pre=True), memb[0:M, :].astype(f32))
        jax.lax.fori_loop(npre, NSEG // UNR, functools.partial(a_steps, pre=False), mem)

        @pl.when(layer == 0)
        def _():
            for c in cp_b[1:]:
                c.wait()
        b1_act(NSEG - 2)
        b1_norm(NSEG - 1)
        b1_dot()
        b1_act(NSEG - 1)
        jax.lax.fori_loop(0, NB, b_phase2, layer)
        return 0

    jax.lax.fori_loop(0, 2, layer_body, 0)

    for i in range(NB):
        pltpu.make_async_copy(ob.at[pl.ds(i * TB, TB), :], out_hbm.at[pl.ds(i * TB, TB), :],
                              sem_o.at[i]).wait()


def pallas_interleave_layers__memory_aug_recurrent_mem_tr__mixer_s_mlp__prompt_kernel(
    A_x: jax.Array,
    A_mem0: jax.Array,
    A_Wq: jax.Array,
    A_Wk: jax.Array,
    A_Wv: jax.Array,
    A_Wo: jax.Array,
    A_seg_len,
    B_x: jax.Array,
    B_w1: jax.Array,
    B_w2: jax.Array,
    B_w3: jax.Array,
    B_w4: jax.Array,
):
    del A_seg_len, B_x

    def wt(w):
        return jnp.transpose(w, (1, 2, 0)).reshape(NH * DH, D)

    any_spec = pl.BlockSpec(memory_space=pl.ANY)
    out = pl.pallas_call(
        _kernel,
        out_shape=jax.ShapeDtypeStruct((S, D), bf16),
        in_specs=[any_spec] * 10,
        out_specs=any_spec,
        scratch_shapes=[
            pltpu.VMEM((NSEG, SEG, D), bf16),
            pltpu.VMEM((NPRE, M, D), bf16),
            pltpu.VMEM((64, D), bf16),
            pltpu.VMEM((NSLOT, 3, PW, D), bf16),
            pltpu.VMEM((NP, D // 2, 3 * PW), jnp.int32),
            pltpu.VMEM((NH * DH // 2, D), jnp.int32),
            pltpu.VMEM((D // 2, D), jnp.int32),
            pltpu.VMEM((D // 2, D), jnp.int32),
            pltpu.VMEM((D // 2, F), jnp.int32),
            pltpu.VMEM((F // 2, D), jnp.int32),
            pltpu.VMEM((S, D), f32),
            pltpu.VMEM((S, D), f32),
            pltpu.VMEM((S, D), f32),
            pltpu.VMEM((S + 32, D), f32),
            pltpu.VMEM((RPRE, D), f32),
            pltpu.VMEM((NP, RPRE, 3 * PW), f32),
            pltpu.VMEM((NP, L, 3 * PW), f32),
            pltpu.VMEM((L, NH * DH), f32),
            pltpu.VMEM((SEG, D), f32),
            pltpu.VMEM((SEG, D), f32),
            pltpu.VMEM((S, D), bf16),
            pltpu.SemaphoreType.DMA((2,)),
            pltpu.SemaphoreType.DMA((NSLOT,)),
            pltpu.SemaphoreType.DMA((5,)),
            pltpu.SemaphoreType.DMA((NB,)),
        ],
        compiler_params=pltpu.CompilerParams(vmem_limit_bytes=120 * 1024 * 1024),
    )(A_x.reshape(NSEG, SEG, D), A_mem0.reshape(M, D), wt(A_Wq), wt(A_Wk), wt(A_Wv),
      A_Wo.reshape(NH * DH, D), B_w1, B_w2, B_w3, B_w4)
    return out.reshape(1, S, D)
```

```python
import functools

import jax
import jax.numpy as jnp
import jax.experimental.pallas as pl
import jax.experimental.pallas.tpu as pltpu

S = 2048
D = 640
NH = 32
DH = 192
M = 8
SEG = 32
L = M + SEG
NSEG = S // SEG
F = 1536
NP = NH // 2
PW = 2 * DH
EPS = 1e-5
SCALE = DH ** -0.5
LOG2E = 1.4426950408889634
PAD = 8
TB = 256
NB = S // TB
NH_B = 4
NPRE = 40
RPRE = NPRE * M
SIN = SEG - M
LN_AT = 5
B1_ACT_AT = 2
B1_NORM_AT = 8
B1_DOTS = ((16, 0, 0, 2), (19, 1, 2, 5))
LAG_OUT = 4
UNR = 2
NSLOT = 4

NT = (((1,), (1,)), ((), ()))
NN = (((1,), (0,)), ((), ()))
f32 = jnp.float32
bf16 = jnp.bfloat16


def _dot(a, b, dims=NN):
    return jax.lax.dot_general(a, b, dims, preferred_element_type=f32)


def _ln(x):
    m = jnp.mean(x, axis=-1, keepdims=True)
    xc = x - m
    v = jnp.mean(xc * xc, axis=-1, keepdims=True)
    return xc * jax.lax.rsqrt(v + EPS)


def _gelu(x):
    return jax.nn.gelu(x, approximate=True)


def _w(ref_val):
    return pltpu.bitcast(ref_val, bf16)


def _blockdiag(x2, lane64):
    z = jnp.zeros((L, 128), x2.dtype)
    a, b, c = x2[:, 0:128], x2[:, 128:256], x2[:, 256:384]
    top = jnp.concatenate([a, jnp.where(lane64, b, 0.0), z], axis=1)
    bot = jnp.concatenate([z, jnp.where(lane64, 0.0, b), c], axis=1)
    return jnp.concatenate([top, bot], axis=0)


def _kernel(x_hbm, mem0_hbm, wq_hbm, wk_hbm, wv_hbm, wo_hbm,
            w1_hbm, w2_hbm, w3_hbm, w4_hbm, out_hbm,
            xb, xl, memb, stage, wqkv, wo_s, w1_s, w2_s, w3_s, w4_s,
            X, H, Y, HB, HL, PRE, qkv_s, o_s, Z, PA, ob,
            sem_x, sem_w, sem_b, sem_o):

    cp_l = pltpu.make_async_copy(x_hbm.at[pl.ds(0, NPRE), pl.ds(SIN, M), :], xl, sem_x.at[0])
    cp_m = pltpu.make_async_copy(mem0_hbm, memb.at[0:M, :], sem_x.at[1])
    cp_l.start()

    XS = NSEG // NP

    def w_copies(hp):
        if isinstance(hp, int):
            r0, s0 = hp * PW, hp * XS
        else:
            r0, s0 = pl.multiple_of(hp * PW, 128), hp * XS
        slot = hp % NSLOT
        cps = [pltpu.make_async_copy(src.at[pl.ds(r0, PW), :], stage.at[slot, a], sem_w.at[slot])
               for a, src in enumerate((wq_hbm, wk_hbm, wv_hbm))]
        cps.append(pltpu.make_async_copy(x_hbm.at[pl.ds(s0, XS)], xb.at[pl.ds(s0, XS)],
                                         sem_w.at[slot]))
        return cps

    for hp in range(2):
        for c in w_copies(hp):
            c.start()
    cp_m.start()

    def wo_copy(hp):
        r0 = hp * DH if isinstance(hp, int) else pl.multiple_of(hp * DH, 64)
        return pltpu.make_async_copy(wo_hbm.bitcast(jnp.int32).at[pl.ds(r0, DH), :],
                                     wo_s.at[pl.ds(r0, DH), :], sem_b.at[0])
    cp_b = [pltpu.make_async_copy(src.bitcast(jnp.int32), dst, sem_b.at[1 + i])
            for i, (src, dst) in enumerate(((w1_hbm, w1_s), (w2_hbm, w2_s),
                                            (w3_hbm, w3_s), (w4_hbm, w4_s)))]

    HB[0:PAD, :] = jnp.zeros((PAD, D), f32)
    HB[PAD + S:PAD + S + PAD, :] = jnp.zeros((PAD, D), f32)
    PA[...] = jnp.zeros((SEG, D), f32)

    cp_l.wait()
    HL[...] = _ln(xl[...].astype(f32).reshape(RPRE, D))

    def tr(hp, _):
        for c in w_copies(hp):
            c.wait()

        @pl.when(hp + 2 < NP)
        def _():
            for c in w_copies(hp + 2):
                c.start()

        wo_copy(hp).start()

        @pl.when(hp == NP - 1)
        def _():
            cp_b[0].start()
        slot = hp % NSLOT
        for a in range(3):
            PRE[hp, :, a * PW:(a + 1) * PW] = _dot(HL[...], stage[slot, a], NT)
            for kt in range(D // 128):
                t = stage[slot, a, :, kt * 128:(kt + 1) * 128].T
                wqkv[hp, kt * 64:(kt + 1) * 64, a * PW:(a + 1) * PW] = pltpu.bitcast(t, jnp.int32)
        X[pl.ds(pl.multiple_of(hp * XS * SEG, XS * SEG), XS * SEG), :] = (
            xb[pl.ds(hp * XS, XS)].astype(f32).reshape(XS * SEG, D))
        return 0
    jax.lax.fori_loop(0, NP, tr, 0)

    cp_m.wait()
    for hp in range(NP):
        wo_copy(hp).wait()
    cp_b[0].wait()
    for c in cp_b[1:]:
        c.start()

    lane64 = jax.lax.broadcasted_iota(jnp.int32, (L, 128), 1) < 64
    ri = jax.lax.broadcasted_iota(jnp.int32, (L, 2 * L), 0)
    ci = jax.lax.broadcasted_iota(jnp.int32, (L, 2 * L), 1)
    first = ci < L
    causal = (ri < M) | (ri >= jnp.where(first, ci, ci - L))

    def seg_rows(s, off=0):
        return pl.ds(pl.multiple_of(s * SEG + off, M), SEG)

    def b1_norm(s):
        y = _ln(X[seg_rows(s), :])
        Y[seg_rows(s), :] = y
        Z[...] = _ln(y)

    def b1_dot(c0=0, c1=D // 128):
        cols = slice(c0 * 128, c1 * 128)
        PA[:, cols] = _dot(Z[...], _w(w1_s[:, cols]))

    def b1_act(s):
        HB[seg_rows(s, PAD), :] = _gelu(PA[...])

    def a_step(s, mem, pre):
        rows = pl.ds(pl.multiple_of(s * SEG, SEG), SEG)
        nin = SIN if pre else SEG
        h = jnp.concatenate([mem, H[pl.ds(pl.multiple_of(s * SEG, SEG), nin), :]], axis=0)
        sc, pr = {}, {}
        acc = [None]

        def st_qkv(hp):
            qkv_s[hp, 0:M + nin, :] = _dot(h, _w(wqkv[hp]))

        def part(hp, a):
            v = qkv_s[hp, 0:M + nin, a * PW:(a + 1) * PW]
            if pre:
                v = jnp.concatenate(
                    [v, PRE[hp, pl.ds(pl.multiple_of(s * M, M), M), a * PW:(a + 1) * PW]], axis=0)
            return v

        def st_qk(hp):
            sc[hp] = _dot(part(hp, 0), _blockdiag(part(hp, 1), lane64), NT)

        def st_softmax(hp):
            v = jnp.where(causal, sc.pop(hp), -1e9 / SCALE)
            m0 = jnp.max(jnp.where(first, v, -jnp.inf), axis=1, keepdims=True)
            m1 = jnp.max(jnp.where(first, -jnp.inf, v), axis=1, keepdims=True)
            e = jnp.exp2((v - jnp.where(first, m0, m1)) * (SCALE * LOG2E))
            pr[hp] = e

        def st_pv(hp):
            e = pr.pop(hp)
            pv = _dot(e, _blockdiag(part(hp, 2), lane64))
            i0 = 1.0 / jnp.sum(jnp.where(first, e, 0.0), axis=1, keepdims=True)
            i1 = 1.0 / jnp.sum(jnp.where(first, 0.0, e), axis=1, keepdims=True)
            o_s[:, hp * PW:(hp + 1) * PW] = jnp.concatenate(
                [pv[:, 0:128] * i0, pv[:, 128:256] * jnp.where(lane64, i0, i1), pv[:, 256:384] * i1],
                axis=1)

        def st_out(hp):
            t = _dot(o_s[:, hp * PW:(hp + 1) * PW], _w(wo_s[hp * DH:(hp + 1) * DH, :]))
            acc[0] = t if acc[0] is None else acc[0] + t

        for i in range(NP + LAG_OUT):
            if i < NP:
                st_qkv(i)
            if i == LN_AT:
                nrows = seg_rows(jnp.minimum(s + 1, NSEG - 1))
                H[nrows, :] = _ln(X[nrows, :])
            if i == B1_ACT_AT:
                b1_act(jnp.maximum(s - 2, 0))
            if i == B1_NORM_AT:
                b1_norm(jnp.maximum(s - 1, 0))
            for (ii, pos, c0, c1) in B1_DOTS:
                if ii == i and pos == 0:
                    b1_dot(c0, c1)
            if 0 <= i - 1 < NP:
                st_qk(i - 1)
            if 0 <= i - 2 < NP:
                st_softmax(i - 2)
            if 0 <= i - 3 < NP:
                st_pv(i - 3)
            if 0 <= i - LAG_OUT < NP:
                st_out(i - LAG_OUT)
            for (ii, pos, c0, c1) in B1_DOTS:
                if ii == i and pos == 1:
                    b1_dot(c0, c1)
        X[rows, :] = X[rows, :] + acc[0][M:, :]
        return acc[0][:M, :]

    TH = TB // NH_B
    lane = jax.lax.broadcasted_iota(jnp.int32, (TH, 128), 1)

    def b_phase2(i, layer):
        r = pl.ds(pl.multiple_of(i * TB, TB), TB)
        rows = [pl.ds(pl.multiple_of(i * TB + u * TH, TH), TH) for u in range(NH_B)]

        def mixed(u):
            win = HB[pl.ds(pl.multiple_of(i * TB + u * TH, TH), TH + 2 * PAD), :]

            def sh(ct, d):
                return win[PAD + d:PAD + d + TH, ct * 128:(ct + 1) * 128]
            return jnp.concatenate([
                sh(0, -1),
                jnp.where(lane < 32, sh(1, -1), sh(1, 1)),
                jnp.where(lane < 64, sh(2, 1), sh(2, -2)),
                jnp.where(lane < 96, sh(3, -2), sh(3, 2)),
                sh(4, 2)], axis=1)

        x1 = [Y[rows[u], :] + _dot(mixed(u), _w(w2_s[...])) for u in range(NH_B)]
        g = [_gelu(_dot(_ln(x1[u]), _w(w3_s[...]))) for u in range(NH_B)]
        for u in range(NH_B):
            xn = X[rows[u], :] + (x1[u] + _dot(g[u], _w(w4_s[...])))
            X[rows[u], :] = xn
            ob[rows[u], :] = xn.astype(bf16)

        @pl.when(layer == 1)
        def _():
            pltpu.make_async_copy(ob.at[r, :], out_hbm.at[r, :], sem_o.at[i]).start()
        return layer

    def layer_body(layer, _):
        H[0:SEG, :] = _ln(X[0:SEG, :])
        def a_steps(j, mem, pre):
            for u in range(UNR):
                mem = a_step(j * UNR + u, mem, pre)
            return mem
        npre = jnp.where(layer == 0, NPRE // UNR, 0)
        mem = jax.lax.fori_loop(0, npre, functools.partial(a_steps, pre=True), memb[0:M, :].astype(f32))
        jax.lax.fori_loop(npre, NSEG // UNR, functools.partial(a_steps, pre=False), mem)

        @pl.when(layer == 0)
        def _():
            for c in cp_b[1:]:
                c.wait()
        b1_act(NSEG - 2)
        b1_norm(NSEG - 1)
        b1_dot()
        b1_act(NSEG - 1)
        jax.lax.fori_loop(0, NB, b_phase2, layer)
        return 0

    jax.lax.fori_loop(0, 2, layer_body, 0)

    for i in range(NB):
        pltpu.make_async_copy(ob.at[pl.ds(i * TB, TB), :], out_hbm.at[pl.ds(i * TB, TB), :],
                              sem_o.at[i]).wait()


def pallas_interleave_layers__memory_aug_recurrent_mem_tr__mixer_s_mlp__prompt_kernel(
    A_x: jax.Array,
    A_mem0: jax.Array,
    A_Wq: jax.Array,
    A_Wk: jax.Array,
    A_Wv: jax.Array,
    A_Wo: jax.Array,
    A_seg_len,
    B_x: jax.Array,
    B_w1: jax.Array,
    B_w2: jax.Array,
    B_w3: jax.Array,
    B_w4: jax.Array,
):
    del A_seg_len, B_x

    def wt(w):
        return jnp.transpose(w, (1, 2, 0)).reshape(NH * DH, D)

    any_spec = pl.BlockSpec(memory_space=pl.ANY)
    out = pl.pallas_call(
        _kernel,
        out_shape=jax.ShapeDtypeStruct((S, D), bf16),
        in_specs=[any_spec] * 10,
        out_specs=any_spec,
        scratch_shapes=[
            pltpu.VMEM((NSEG, SEG, D), bf16),
            pltpu.VMEM((NPRE, M, D), bf16),
            pltpu.VMEM((64, D), bf16),
            pltpu.VMEM((NSLOT, 3, PW, D), bf16),
            pltpu.VMEM((NP, D // 2, 3 * PW), jnp.int32),
            pltpu.VMEM((NH * DH // 2, D), jnp.int32),
            pltpu.VMEM((D // 2, D), jnp.int32),
            pltpu.VMEM((D // 2, D), jnp.int32),
            pltpu.VMEM((D // 2, F), jnp.int32),
            pltpu.VMEM((F // 2, D), jnp.int32),
            pltpu.VMEM((S, D), f32),
            pltpu.VMEM((S, D), f32),
            pltpu.VMEM((S, D), f32),
            pltpu.VMEM((S + 32, D), f32),
            pltpu.VMEM((RPRE, D), f32),
            pltpu.VMEM((NP, RPRE, 3 * PW), f32),
            pltpu.VMEM((NP, L, 3 * PW), f32),
            pltpu.VMEM((L, NH * DH), f32),
            pltpu.VMEM((SEG, D), f32),
            pltpu.VMEM((SEG, D), f32),
            pltpu.VMEM((S, D), bf16),
            pltpu.SemaphoreType.DMA((2,)),
            pltpu.SemaphoreType.DMA((NSLOT,)),
            pltpu.SemaphoreType.DMA((5,)),
            pltpu.SemaphoreType.DMA((NB,)),
        ],
        compiler_params=pltpu.CompilerParams(vmem_limit_bytes=120 * 1024 * 1024),
    )(A_x.reshape(NSEG, SEG, D), A_mem0.reshape(M, D), wt(A_Wq), wt(A_Wk), wt(A_Wv),
      A_Wo.reshape(NH * DH, D), B_w1, B_w2, B_w3, B_w4)
    return out.reshape(1, S, D)
```

```python
import functools

import jax
import jax.numpy as jnp
import jax.experimental.pallas as pl
import jax.experimental.pallas.tpu as pltpu

S = 2048
D = 640
NH = 32
DH = 192
M = 8
SEG = 32
L = M + SEG
NSEG = S // SEG
F = 1536
NP = NH // 2
PW = 2 * DH
EPS = 1e-5
SCALE = DH ** -0.5
LOG2E = 1.4426950408889634
PAD = 8
TB = 256
NB = S // TB
NH_B = 4
NPRE = 40
RPRE = NPRE * M
SIN = SEG - M
LN_AT = 5
B1_ACT_AT = 2
B1_NORM_AT = 8
B1_DOTS = ((16, 0, 0, 2), (19, 1, 2, 5))
LAG_OUT = 4
UNR = 2
NSLOT = 4

NT = (((1,), (1,)), ((), ()))
NN = (((1,), (0,)), ((), ()))
f32 = jnp.float32
bf16 = jnp.bfloat16


def _dot(a, b, dims=NN):
    return jax.lax.dot_general(a, b, dims, preferred_element_type=f32)


def _ln(x):
    m = jnp.mean(x, axis=-1, keepdims=True)
    xc = x - m
    v = jnp.mean(xc * xc, axis=-1, keepdims=True)
    return xc * jax.lax.rsqrt(v + EPS)


def _gelu(x):
    return jax.nn.gelu(x, approximate=True)


def _w(ref_val):
    return pltpu.bitcast(ref_val, bf16)


def _blockdiag(x2, lane64):
    z = jnp.zeros((L, 128), x2.dtype)
    a, b, c = x2[:, 0:128], x2[:, 128:256], x2[:, 256:384]
    top = jnp.concatenate([a, jnp.where(lane64, b, 0.0), z], axis=1)
    bot = jnp.concatenate([z, jnp.where(lane64, 0.0, b), c], axis=1)
    return jnp.concatenate([top, bot], axis=0)


def _kernel(x_hbm, mem0_hbm, wq_hbm, wk_hbm, wv_hbm, wo_hbm,
            w1_hbm, w2_hbm, w3_hbm, w4_hbm, out_hbm,
            xb, xl, memb, stage, wqkv, wo_s, w1_s, w2_s, w3_s, w4_s,
            X, H, Y, HB, HL, PRE, qkv_s, o_s, Z, PA, ob,
            sem_x, sem_w, sem_b, sem_o):

    cp_l = pltpu.make_async_copy(x_hbm.at[pl.ds(0, NPRE), pl.ds(SIN, M), :], xl, sem_x.at[0])
    cp_m = pltpu.make_async_copy(mem0_hbm, memb.at[0:M, :], sem_x.at[1])
    cp_l.start()

    XS = NSEG // NP

    def w_copies(hp):
        if isinstance(hp, int):
            r0, s0 = hp * PW, hp * XS
        else:
            r0, s0 = pl.multiple_of(hp * PW, 128), hp * XS
        slot = hp % NSLOT
        cps = [pltpu.make_async_copy(src.at[pl.ds(r0, PW), :], stage.at[slot, a], sem_w.at[slot])
               for a, src in enumerate((wq_hbm, wk_hbm, wv_hbm))]
        cps.append(pltpu.make_async_copy(x_hbm.at[pl.ds(s0, XS)], xb.at[pl.ds(s0, XS)],
                                         sem_w.at[slot]))
        return cps

    for hp in range(2):
        for c in w_copies(hp):
            c.start()
    cp_m.start()

    def wo_copy(hp):
        r0 = hp * DH if isinstance(hp, int) else pl.multiple_of(hp * DH, 64)
        return pltpu.make_async_copy(wo_hbm.bitcast(jnp.int32).at[pl.ds(r0, DH), :],
                                     wo_s.at[pl.ds(r0, DH), :], sem_b.at[0])
    cp_b = [pltpu.make_async_copy(src.bitcast(jnp.int32), dst, sem_b.at[1 + i])
            for i, (src, dst) in enumerate(((w1_hbm, w1_s), (w2_hbm, w2_s),
                                            (w3_hbm, w3_s), (w4_hbm, w4_s)))]

    HB[0:PAD, :] = jnp.zeros((PAD, D), f32)
    HB[PAD + S:PAD + S + PAD, :] = jnp.zeros((PAD, D), f32)
    PA[...] = jnp.zeros((SEG, D), f32)

    cp_l.wait()
    HL[...] = _ln(xl[...].astype(f32).reshape(RPRE, D))

    def tr(hp, _):
        for c in w_copies(hp):
            c.wait()

        @pl.when(hp + 2 < NP)
        def _():
            for c in w_copies(hp + 2):
                c.start()

        wo_copy(hp).start()

        @pl.when(hp == NP - 1)
        def _():
            cp_b[0].start()
        slot = hp % NSLOT
        for a in range(3):
            PRE[hp, :, a * PW:(a + 1) * PW] = _dot(HL[...], stage[slot, a], NT)
            for kt in range(D // 128):
                t = stage[slot, a, :, kt * 128:(kt + 1) * 128].T
                wqkv[hp, kt * 64:(kt + 1) * 64, a * PW:(a + 1) * PW] = pltpu.bitcast(t, jnp.int32)
        X[pl.ds(pl.multiple_of(hp * XS * SEG, XS * SEG), XS * SEG), :] = (
            xb[pl.ds(hp * XS, XS)].astype(f32).reshape(XS * SEG, D))
        return 0
    jax.lax.fori_loop(0, NP, tr, 0)

    cp_m.wait()
    for hp in range(NP):
        wo_copy(hp).wait()
    cp_b[0].wait()
    for c in cp_b[1:]:
        c.start()

    lane64 = jax.lax.broadcasted_iota(jnp.int32, (L, 128), 1) < 64
    ri = jax.lax.broadcasted_iota(jnp.int32, (L, 2 * L), 0)
    ci = jax.lax.broadcasted_iota(jnp.int32, (L, 2 * L), 1)
    first = ci < L
    causal = (ri < M) | (ri >= jnp.where(first, ci, ci - L))

    def seg_rows(s, off=0):
        return pl.ds(pl.multiple_of(s * SEG + off, M), SEG)

    def b1_norm(s):
        y = _ln(X[seg_rows(s), :])
        Y[seg_rows(s), :] = y
        Z[...] = _ln(y)

    def b1_dot(c0=0, c1=D // 128):
        cols = slice(c0 * 128, c1 * 128)
        PA[:, cols] = _dot(Z[...], _w(w1_s[:, cols]))

    def b1_act(s):
        HB[seg_rows(s, PAD), :] = _gelu(PA[...])

    def a_step(s, mem, pre):
        rows = pl.ds(pl.multiple_of(s * SEG, SEG), SEG)
        nin = SIN if pre else SEG
        h = jnp.concatenate([mem, H[pl.ds(pl.multiple_of(s * SEG, SEG), nin), :]], axis=0)
        sc, pr = {}, {}
        acc = [None]

        def st_qkv(hp):
            qkv_s[hp, 0:M + nin, :] = _dot(h, _w(wqkv[hp]))

        def part(hp, a):
            v = qkv_s[hp, 0:M + nin, a * PW:(a + 1) * PW]
            if pre:
                v = jnp.concatenate(
                    [v, PRE[hp, pl.ds(pl.multiple_of(s * M, M), M), a * PW:(a + 1) * PW]], axis=0)
            return v

        def st_qk(hp):
            sc[hp] = _dot(part(hp, 0), _blockdiag(part(hp, 1), lane64), NT)

        def st_softmax(hp):
            v = jnp.where(causal, sc.pop(hp), -1e9 / SCALE)
            m0 = jnp.max(jnp.where(first, v, -jnp.inf), axis=1, keepdims=True)
            m1 = jnp.max(jnp.where(first, -jnp.inf, v), axis=1, keepdims=True)
            e = jnp.exp2((v - jnp.where(first, m0, m1)) * (SCALE * LOG2E))
            pr[hp] = e

        def st_pv(hp):
            e = pr.pop(hp)
            pv = _dot(e, _blockdiag(part(hp, 2), lane64))
            i0 = 1.0 / jnp.sum(jnp.where(first, e, 0.0), axis=1, keepdims=True)
            i1 = 1.0 / jnp.sum(jnp.where(first, 0.0, e), axis=1, keepdims=True)
            o_s[:, hp * PW:(hp + 1) * PW] = jnp.concatenate(
                [pv[:, 0:128] * i0, pv[:, 128:256] * jnp.where(lane64, i0, i1), pv[:, 256:384] * i1],
                axis=1)

        def st_out(hp):
            t = _dot(o_s[:, hp * PW:(hp + 1) * PW], _w(wo_s[hp * DH:(hp + 1) * DH, :]))
            acc[0] = t if acc[0] is None else acc[0] + t

        for i in range(NP + LAG_OUT):
            if i < NP:
                st_qkv(i)
            if i == LN_AT:
                nrows = seg_rows(jnp.minimum(s + 1, NSEG - 1))
                H[nrows, :] = _ln(X[nrows, :])
            if i == B1_ACT_AT:
                b1_act(jnp.maximum(s - 2, 0))
            if i == B1_NORM_AT:
                b1_norm(jnp.maximum(s - 1, 0))
            for (ii, pos, c0, c1) in B1_DOTS:
                if ii == i and pos == 0:
                    b1_dot(c0, c1)
            if 0 <= i - 1 < NP:
                st_qk(i - 1)
            if 0 <= i - 2 < NP:
                st_softmax(i - 2)
            if 0 <= i - 3 < NP:
                st_pv(i - 3)
            if 0 <= i - LAG_OUT < NP:
                st_out(i - LAG_OUT)
            for (ii, pos, c0, c1) in B1_DOTS:
                if ii == i and pos == 1:
                    b1_dot(c0, c1)
        X[rows, :] = X[rows, :] + acc[0][M:, :]
        return acc[0][:M, :]

    TH = TB // NH_B
    lane = jax.lax.broadcasted_iota(jnp.int32, (TH, 128), 1)

    def b_phase2(i, layer, tail=False):
        mo = (lambda v, m: v) if isinstance(i, int) else pl.multiple_of
        r = pl.ds(mo(i * TB, TB), TB)
        rows = [pl.ds(mo(i * TB + u * TH, TH), TH) for u in range(NH_B)]

        def mixed(u):
            win = HB[pl.ds(mo(i * TB + u * TH, TH), TH + 2 * PAD), :]

            def sh(ct, d):
                return win[PAD + d:PAD + d + TH, ct * 128:(ct + 1) * 128]
            return jnp.concatenate([
                sh(0, -1),
                jnp.where(lane < 32, sh(1, -1), sh(1, 1)),
                jnp.where(lane < 64, sh(2, 1), sh(2, -2)),
                jnp.where(lane < 96, sh(3, -2), sh(3, 2)),
                sh(4, 2)], axis=1)

        if tail:
            b1_act(NSEG - 2)
            b1_norm(NSEG - 1)
        x1 = [Y[rows[u], :] + _dot(mixed(u), _w(w2_s[...])) for u in range(NH_B)]
        if tail:
            b1_dot()
            b1_act(NSEG - 1)
        g = [_gelu(_dot(_ln(x1[u]), _w(w3_s[...]))) for u in range(NH_B)]
        for u in range(NH_B):
            xn = X[rows[u], :] + (x1[u] + _dot(g[u], _w(w4_s[...])))
            X[rows[u], :] = xn
            ob[rows[u], :] = xn.astype(bf16)

        @pl.when(layer == 1)
        def _():
            pltpu.make_async_copy(ob.at[r, :], out_hbm.at[r, :], sem_o.at[i]).start()
        return layer

    def layer_body(layer, _):
        H[0:SEG, :] = _ln(X[0:SEG, :])
        def a_steps(j, mem, pre):
            for u in range(UNR):
                mem = a_step(j * UNR + u, mem, pre)
            return mem
        npre = jnp.where(layer == 0, NPRE // UNR, 0)
        mem = jax.lax.fori_loop(0, npre, functools.partial(a_steps, pre=True), memb[0:M, :].astype(f32))
        jax.lax.fori_loop(npre, NSEG // UNR, functools.partial(a_steps, pre=False), mem)

        @pl.when(layer == 0)
        def _():
            for c in cp_b[1:]:
                c.wait()
        b_phase2(0, layer, tail=True)
        jax.lax.fori_loop(1, NB, b_phase2, layer)
        return 0

    jax.lax.fori_loop(0, 2, layer_body, 0)

    for i in range(NB):
        pltpu.make_async_copy(ob.at[pl.ds(i * TB, TB), :], out_hbm.at[pl.ds(i * TB, TB), :],
                              sem_o.at[i]).wait()


def pallas_interleave_layers__memory_aug_recurrent_mem_tr__mixer_s_mlp__prompt_kernel(
    A_x: jax.Array,
    A_mem0: jax.Array,
    A_Wq: jax.Array,
    A_Wk: jax.Array,
    A_Wv: jax.Array,
    A_Wo: jax.Array,
    A_seg_len,
    B_x: jax.Array,
    B_w1: jax.Array,
    B_w2: jax.Array,
    B_w3: jax.Array,
    B_w4: jax.Array,
):
    del A_seg_len, B_x

    def wt(w):
        return jnp.transpose(w, (1, 2, 0)).reshape(NH * DH, D)

    any_spec = pl.BlockSpec(memory_space=pl.ANY)
    out = pl.pallas_call(
        _kernel,
        out_shape=jax.ShapeDtypeStruct((S, D), bf16),
        in_specs=[any_spec] * 10,
        out_specs=any_spec,
        scratch_shapes=[
            pltpu.VMEM((NSEG, SEG, D), bf16),
            pltpu.VMEM((NPRE, M, D), bf16),
            pltpu.VMEM((64, D), bf16),
            pltpu.VMEM((NSLOT, 3, PW, D), bf16),
            pltpu.VMEM((NP, D // 2, 3 * PW), jnp.int32),
            pltpu.VMEM((NH * DH // 2, D), jnp.int32),
            pltpu.VMEM((D // 2, D), jnp.int32),
            pltpu.VMEM((D // 2, D), jnp.int32),
            pltpu.VMEM((D // 2, F), jnp.int32),
            pltpu.VMEM((F // 2, D), jnp.int32),
            pltpu.VMEM((S, D), f32),
            pltpu.VMEM((S, D), f32),
            pltpu.VMEM((S, D), f32),
            pltpu.VMEM((S + 32, D), f32),
            pltpu.VMEM((RPRE, D), f32),
            pltpu.VMEM((NP, RPRE, 3 * PW), f32),
            pltpu.VMEM((NP, L, 3 * PW), f32),
            pltpu.VMEM((L, NH * DH), f32),
            pltpu.VMEM((SEG, D), f32),
            pltpu.VMEM((SEG, D), f32),
            pltpu.VMEM((S, D), bf16),
            pltpu.SemaphoreType.DMA((2,)),
            pltpu.SemaphoreType.DMA((NSLOT,)),
            pltpu.SemaphoreType.DMA((5,)),
            pltpu.SemaphoreType.DMA((NB,)),
        ],
        compiler_params=pltpu.CompilerParams(vmem_limit_bytes=120 * 1024 * 1024),
    )(A_x.reshape(NSEG, SEG, D), A_mem0.reshape(M, D), wt(A_Wq), wt(A_Wk), wt(A_Wv),
      A_Wo.reshape(NH * DH, D), B_w1, B_w2, B_w3, B_w4)
    return out.reshape(1, S, D)
```

```python
import functools

import jax
import jax.numpy as jnp
import jax.experimental.pallas as pl
import jax.experimental.pallas.tpu as pltpu

S = 2048
D = 640
NH = 32
DH = 192
M = 8
SEG = 32
L = M + SEG
NSEG = S // SEG
F = 1536
NP = NH // 2
PW = 2 * DH
EPS = 1e-5
SCALE = DH ** -0.5
LOG2E = 1.4426950408889634
PAD = 8
TB = 256
NB = S // TB
NH_B = 4
NPRE = 40
RPRE = NPRE * M
SIN = SEG - M
LN_AT = 5
B1_ACT_AT = 2
B1_NORM_AT = 8
B1_DOTS = ((16, 0, 0, 2), (19, 1, 2, 5))
LAG_OUT = 4
ORDER = ('p02', 'b0', 'qk', 'pv', 'p23', 'out', 'b1')
UNR = 2
NSLOT = 4

NT = (((1,), (1,)), ((), ()))
NN = (((1,), (0,)), ((), ()))
f32 = jnp.float32
bf16 = jnp.bfloat16


def _dot(a, b, dims=NN):
    return jax.lax.dot_general(a, b, dims, preferred_element_type=f32)


def _ln(x):
    m = jnp.mean(x, axis=-1, keepdims=True)
    xc = x - m
    v = jnp.mean(xc * xc, axis=-1, keepdims=True)
    return xc * jax.lax.rsqrt(v + EPS)


def _gelu(x):
    return jax.nn.gelu(x, approximate=True)


def _w(ref_val):
    return pltpu.bitcast(ref_val, bf16)


def _blockdiag(x2, lane64):
    z = jnp.zeros((L, 128), x2.dtype)
    a, b, c = x2[:, 0:128], x2[:, 128:256], x2[:, 256:384]
    top = jnp.concatenate([a, jnp.where(lane64, b, 0.0), z], axis=1)
    bot = jnp.concatenate([z, jnp.where(lane64, 0.0, b), c], axis=1)
    return jnp.concatenate([top, bot], axis=0)


def _kernel(x_hbm, mem0_hbm, wq_hbm, wk_hbm, wv_hbm, wo_hbm,
            w1_hbm, w2_hbm, w3_hbm, w4_hbm, out_hbm,
            xb, xl, memb, stage, wqkv, wo_s, w1_s, w2_s, w3_s, w4_s,
            X, H, Y, HB, HL, PRE, qkv_s, o_s, Z, PA, ob,
            sem_x, sem_w, sem_b, sem_o):

    cp_l = pltpu.make_async_copy(x_hbm.at[pl.ds(0, NPRE), pl.ds(SIN, M), :], xl, sem_x.at[0])
    cp_m = pltpu.make_async_copy(mem0_hbm, memb.at[0:M, :], sem_x.at[1])
    cp_l.start()

    XS = NSEG // NP

    def w_copies(hp):
        if isinstance(hp, int):
            r0, s0 = hp * PW, hp * XS
        else:
            r0, s0 = pl.multiple_of(hp * PW, 128), hp * XS
        slot = hp % NSLOT
        cps = [pltpu.make_async_copy(src.at[pl.ds(r0, PW), :], stage.at[slot, a], sem_w.at[slot])
               for a, src in enumerate((wq_hbm, wk_hbm, wv_hbm))]
        cps.append(pltpu.make_async_copy(x_hbm.at[pl.ds(s0, XS)], xb.at[pl.ds(s0, XS)],
                                         sem_w.at[slot]))
        return cps

    for hp in range(2):
        for c in w_copies(hp):
            c.start()
    cp_m.start()

    def wo_copy(hp):
        r0 = hp * DH if isinstance(hp, int) else pl.multiple_of(hp * DH, 64)
        return pltpu.make_async_copy(wo_hbm.bitcast(jnp.int32).at[pl.ds(r0, DH), :],
                                     wo_s.at[pl.ds(r0, DH), :], sem_b.at[0])
    cp_b = [pltpu.make_async_copy(src.bitcast(jnp.int32), dst, sem_b.at[1 + i])
            for i, (src, dst) in enumerate(((w1_hbm, w1_s), (w2_hbm, w2_s),
                                            (w3_hbm, w3_s), (w4_hbm, w4_s)))]

    HB[0:PAD, :] = jnp.zeros((PAD, D), f32)
    HB[PAD + S:PAD + S + PAD, :] = jnp.zeros((PAD, D), f32)
    PA[...] = jnp.zeros((SEG, D), f32)

    cp_l.wait()
    HL[...] = _ln(xl[...].astype(f32).reshape(RPRE, D))

    def tr(hp, _):
        for c in w_copies(hp):
            c.wait()

        @pl.when(hp + 2 < NP)
        def _():
            for c in w_copies(hp + 2):
                c.start()

        wo_copy(hp).start()

        @pl.when(hp == NP - 1)
        def _():
            cp_b[0].start()
        slot = hp % NSLOT
        for a in range(3):
            PRE[hp, :, a * PW:(a + 1) * PW] = _dot(HL[...], stage[slot, a], NT)
            for kt in range(D // 128):
                t = stage[slot, a, :, kt * 128:(kt + 1) * 128].T
                wqkv[hp, kt * 64:(kt + 1) * 64, a * PW:(a + 1) * PW] = pltpu.bitcast(t, jnp.int32)
        X[pl.ds(pl.multiple_of(hp * XS * SEG, XS * SEG), XS * SEG), :] = (
            xb[pl.ds(hp * XS, XS)].astype(f32).reshape(XS * SEG, D))
        return 0
    jax.lax.fori_loop(0, NP, tr, 0)

    cp_m.wait()
    for hp in range(NP):
        wo_copy(hp).wait()
    cp_b[0].wait()
    for c in cp_b[1:]:
        c.start()

    lane64 = jax.lax.broadcasted_iota(jnp.int32, (L, 128), 1) < 64
    ri = jax.lax.broadcasted_iota(jnp.int32, (L, 2 * L), 0)
    ci = jax.lax.broadcasted_iota(jnp.int32, (L, 2 * L), 1)
    first = ci < L
    causal = (ri < M) | (ri >= jnp.where(first, ci, ci - L))

    def seg_rows(s, off=0):
        return pl.ds(pl.multiple_of(s * SEG + off, M), SEG)

    def b1_norm(s):
        y = _ln(X[seg_rows(s), :])
        Y[seg_rows(s), :] = y
        Z[...] = _ln(y)

    def b1_dot(c0=0, c1=D // 128):
        cols = slice(c0 * 128, c1 * 128)
        PA[:, cols] = _dot(Z[...], _w(w1_s[:, cols]))

    def b1_act(s):
        HB[seg_rows(s, PAD), :] = _gelu(PA[...])

    def a_step(s, mem, pre):
        rows = pl.ds(pl.multiple_of(s * SEG, SEG), SEG)
        nin = SIN if pre else SEG
        h = jnp.concatenate([mem, H[pl.ds(pl.multiple_of(s * SEG, SEG), nin), :]], axis=0)
        sc, pr = {}, {}
        acc = [None]

        def st_qkv(hp):
            qkv_s[hp, 0:M + nin, :] = _dot(h, _w(wqkv[hp]))

        def part(hp, a):
            v = qkv_s[hp, 0:M + nin, a * PW:(a + 1) * PW]
            if pre:
                v = jnp.concatenate(
                    [v, PRE[hp, pl.ds(pl.multiple_of(s * M, M), M), a * PW:(a + 1) * PW]], axis=0)
            return v

        def st_qk(hp):
            sc[hp] = _dot(part(hp, 0), _blockdiag(part(hp, 1), lane64), NT)

        def st_softmax(hp):
            v = jnp.where(causal, sc.pop(hp), -1e9 / SCALE)
            m0 = jnp.max(jnp.where(first, v, -jnp.inf), axis=1, keepdims=True)
            m1 = jnp.max(jnp.where(first, -jnp.inf, v), axis=1, keepdims=True)
            e = jnp.exp2((v - jnp.where(first, m0, m1)) * (SCALE * LOG2E))
            pr[hp] = e

        def st_pv(hp):
            e = pr.pop(hp)
            pv = _dot(e, _blockdiag(part(hp, 2), lane64))
            i0 = 1.0 / jnp.sum(jnp.where(first, e, 0.0), axis=1, keepdims=True)
            i1 = 1.0 / jnp.sum(jnp.where(first, 0.0, e), axis=1, keepdims=True)
            o_s[:, hp * PW:(hp + 1) * PW] = jnp.concatenate(
                [pv[:, 0:128] * i0, pv[:, 128:256] * jnp.where(lane64, i0, i1), pv[:, 256:384] * i1],
                axis=1)

        def st_out(hp):
            t = _dot(o_s[:, hp * PW:(hp + 1) * PW], _w(wo_s[hp * DH:(hp + 1) * DH, :]))
            acc[0] = t if acc[0] is None else acc[0] + t

        def st_proj(hp, a0, a1):
            cols = slice(a0 * PW, a1 * PW)
            qkv_s[hp, 0:M + nin, cols] = _dot(h, _w(wqkv[hp, :, cols]))

        for i in range(NP + LAG_OUT):
            if i == LN_AT:
                nrows = seg_rows(jnp.minimum(s + 1, NSEG - 1))
                H[nrows, :] = _ln(X[nrows, :])
            if i == B1_ACT_AT:
                b1_act(jnp.maximum(s - 2, 0))
            if i == B1_NORM_AT:
                b1_norm(jnp.maximum(s - 1, 0))
            if 0 <= i - 2 < NP:
                st_softmax(i - 2)
            for name in ORDER:
                if name == "b0" or name == "b1":
                    for (ii, pos, c0, c1) in B1_DOTS:
                        if ii == i and pos == int(name[1]):
                            b1_dot(c0, c1)
                elif name == "qk":
                    if 0 <= i - 1 < NP:
                        st_qk(i - 1)
                elif name == "pv":
                    if 0 <= i - 3 < NP:
                        st_pv(i - 3)
                elif name == "out":
                    if 0 <= i - LAG_OUT < NP:
                        st_out(i - LAG_OUT)
                elif i < NP:
                    st_proj(i, int(name[1]), int(name[2]))
        X[rows, :] = X[rows, :] + acc[0][M:, :]
        return acc[0][:M, :]

    TH = TB // NH_B
    lane = jax.lax.broadcasted_iota(jnp.int32, (TH, 128), 1)

    def b_phase2(i, layer, tail=False):
        mo = (lambda v, m: v) if isinstance(i, int) else pl.multiple_of
        r = pl.ds(mo(i * TB, TB), TB)
        rows = [pl.ds(mo(i * TB + u * TH, TH), TH) for u in range(NH_B)]

        def mixed(u):
            win = HB[pl.ds(mo(i * TB + u * TH, TH), TH + 2 * PAD), :]

            def sh(ct, d):
                return win[PAD + d:PAD + d + TH, ct * 128:(ct + 1) * 128]
            return jnp.concatenate([
                sh(0, -1),
                jnp.where(lane < 32, sh(1, -1), sh(1, 1)),
                jnp.where(lane < 64, sh(2, 1), sh(2, -2)),
                jnp.where(lane < 96, sh(3, -2), sh(3, 2)),
                sh(4, 2)], axis=1)

        if tail:
            b1_act(NSEG - 2)
            b1_norm(NSEG - 1)
        x1 = [Y[rows[u], :] + _dot(mixed(u), _w(w2_s[...])) for u in range(NH_B)]
        if tail:
            b1_dot()
            b1_act(NSEG - 1)
        g = [_gelu(_dot(_ln(x1[u]), _w(w3_s[...]))) for u in range(NH_B)]
        for u in range(NH_B):
            xn = X[rows[u], :] + (x1[u] + _dot(g[u], _w(w4_s[...])))
            X[rows[u], :] = xn
            ob[rows[u], :] = xn.astype(bf16)

        @pl.when(layer == 1)
        def _():
            pltpu.make_async_copy(ob.at[r, :], out_hbm.at[r, :], sem_o.at[i]).start()
        return layer

    def layer_body(layer, _):
        H[0:SEG, :] = _ln(X[0:SEG, :])
        def a_steps(j, mem, pre):
            for u in range(UNR):
                mem = a_step(j * UNR + u, mem, pre)
            return mem
        npre = jnp.where(layer == 0, NPRE // UNR, 0)
        mem = jax.lax.fori_loop(0, npre, functools.partial(a_steps, pre=True), memb[0:M, :].astype(f32))
        jax.lax.fori_loop(npre, NSEG // UNR, functools.partial(a_steps, pre=False), mem)

        @pl.when(layer == 0)
        def _():
            for c in cp_b[1:]:
                c.wait()
        b_phase2(0, layer, tail=True)
        jax.lax.fori_loop(1, NB, b_phase2, layer)
        return 0

    jax.lax.fori_loop(0, 2, layer_body, 0)

    for i in range(NB):
        pltpu.make_async_copy(ob.at[pl.ds(i * TB, TB), :], out_hbm.at[pl.ds(i * TB, TB), :],
                              sem_o.at[i]).wait()


def pallas_interleave_layers__memory_aug_recurrent_mem_tr__mixer_s_mlp__prompt_kernel(
    A_x: jax.Array,
    A_mem0: jax.Array,
    A_Wq: jax.Array,
    A_Wk: jax.Array,
    A_Wv: jax.Array,
    A_Wo: jax.Array,
    A_seg_len,
    B_x: jax.Array,
    B_w1: jax.Array,
    B_w2: jax.Array,
    B_w3: jax.Array,
    B_w4: jax.Array,
):
    del A_seg_len, B_x

    def wt(w):
        return jnp.transpose(w, (1, 2, 0)).reshape(NH * DH, D)

    any_spec = pl.BlockSpec(memory_space=pl.ANY)
    out = pl.pallas_call(
        _kernel,
        out_shape=jax.ShapeDtypeStruct((S, D), bf16),
        in_specs=[any_spec] * 10,
        out_specs=any_spec,
        scratch_shapes=[
            pltpu.VMEM((NSEG, SEG, D), bf16),
            pltpu.VMEM((NPRE, M, D), bf16),
            pltpu.VMEM((64, D), bf16),
            pltpu.VMEM((NSLOT, 3, PW, D), bf16),
            pltpu.VMEM((NP, D // 2, 3 * PW), jnp.int32),
            pltpu.VMEM((NH * DH // 2, D), jnp.int32),
            pltpu.VMEM((D // 2, D), jnp.int32),
            pltpu.VMEM((D // 2, D), jnp.int32),
            pltpu.VMEM((D // 2, F), jnp.int32),
            pltpu.VMEM((F // 2, D), jnp.int32),
            pltpu.VMEM((S, D), f32),
            pltpu.VMEM((S, D), f32),
            pltpu.VMEM((S, D), f32),
            pltpu.VMEM((S + 32, D), f32),
            pltpu.VMEM((RPRE, D), f32),
            pltpu.VMEM((NP, RPRE, 3 * PW), f32),
            pltpu.VMEM((NP, L, 3 * PW), f32),
            pltpu.VMEM((L, NH * DH), f32),
            pltpu.VMEM((SEG, D), f32),
            pltpu.VMEM((SEG, D), f32),
            pltpu.VMEM((S, D), bf16),
            pltpu.SemaphoreType.DMA((2,)),
            pltpu.SemaphoreType.DMA((NSLOT,)),
            pltpu.SemaphoreType.DMA((5,)),
            pltpu.SemaphoreType.DMA((NB,)),
        ],
        compiler_params=pltpu.CompilerParams(vmem_limit_bytes=120 * 1024 * 1024),
    )(A_x.reshape(NSEG, SEG, D), A_mem0.reshape(M, D), wt(A_Wq), wt(A_Wk), wt(A_Wv),
      A_Wo.reshape(NH * DH, D), B_w1, B_w2, B_w3, B_w4)
    return out.reshape(1, S, D)
```

```python
import functools

import jax
import jax.numpy as jnp
import jax.experimental.pallas as pl
import jax.experimental.pallas.tpu as pltpu

S = 2048
D = 640
NH = 32
DH = 192
M = 8
SEG = 32
L = M + SEG
NSEG = S // SEG
F = 1536
NP = NH // 2
PW = 2 * DH
EPS = 1e-5
SCALE = DH ** -0.5
LOG2E = 1.4426950408889634
PAD = 8
TB = 256
NB = S // TB
NH_B = 4
NPRE = 40
RPRE = NPRE * M
SIN = SEG - M
UNR = 2
NSLOT = 4

NT = (((1,), (1,)), ((), ()))
NN = (((1,), (0,)), ((), ()))
f32 = jnp.float32
bf16 = jnp.bfloat16


def _dot(a, b, dims=NN):
    return jax.lax.dot_general(a, b, dims, preferred_element_type=f32)


def _ln(x):
    m = jnp.mean(x, axis=-1, keepdims=True)
    xc = x - m
    v = jnp.mean(xc * xc, axis=-1, keepdims=True)
    return xc * jax.lax.rsqrt(v + EPS)


def _gelu(x):
    return jax.nn.gelu(x, approximate=True)


def _w(ref_val):
    return pltpu.bitcast(ref_val, bf16)


def _blockdiag(x2, lane64):
    z = jnp.zeros((L, 128), x2.dtype)
    a, b, c = x2[:, 0:128], x2[:, 128:256], x2[:, 256:384]
    top = jnp.concatenate([a, jnp.where(lane64, b, 0.0), z], axis=1)
    bot = jnp.concatenate([z, jnp.where(lane64, 0.0, b), c], axis=1)
    return jnp.concatenate([top, bot], axis=0)


def _kernel(x_hbm, mem0_hbm, wq_hbm, wk_hbm, wv_hbm, wo_hbm,
            w1_hbm, w2_hbm, w3_hbm, w4_hbm, out_hbm,
            xb, xl, memb, stage, wqkv, wo_s, w1_s, w2_s, w3_s, w4_s,
            X, H, Y, HB, HL, PRE, qkv_s, o_s, Z, PA, ob,
            sem_x, sem_w, sem_b, sem_o):

    cp_l = pltpu.make_async_copy(x_hbm.at[pl.ds(0, NPRE), pl.ds(SIN, M), :], xl, sem_x.at[0])
    cp_m = pltpu.make_async_copy(mem0_hbm, memb.at[0:M, :], sem_x.at[1])
    cp_l.start()

    XS = NSEG // NP

    def w_copies(hp):
        if isinstance(hp, int):
            r0, s0 = hp * PW, hp * XS
        else:
            r0, s0 = pl.multiple_of(hp * PW, 128), hp * XS
        slot = hp % NSLOT
        cps = [pltpu.make_async_copy(src.at[pl.ds(r0, PW), :], stage.at[slot, a], sem_w.at[slot])
               for a, src in enumerate((wq_hbm, wk_hbm, wv_hbm))]
        cps.append(pltpu.make_async_copy(x_hbm.at[pl.ds(s0, XS)], xb.at[pl.ds(s0, XS)],
                                         sem_w.at[slot]))
        return cps

    for hp in range(2):
        for c in w_copies(hp):
            c.start()
    cp_m.start()

    def wo_copy(hp):
        r0 = hp * DH if isinstance(hp, int) else pl.multiple_of(hp * DH, 64)
        return pltpu.make_async_copy(wo_hbm.bitcast(jnp.int32).at[pl.ds(r0, DH), :],
                                     wo_s.at[pl.ds(r0, DH), :], sem_b.at[0])
    cp_b = [pltpu.make_async_copy(src.bitcast(jnp.int32), dst, sem_b.at[1 + i])
            for i, (src, dst) in enumerate(((w1_hbm, w1_s), (w2_hbm, w2_s),
                                            (w3_hbm, w3_s), (w4_hbm, w4_s)))]

    HB[0:PAD, :] = jnp.zeros((PAD, D), f32)
    HB[PAD + S:PAD + S + PAD, :] = jnp.zeros((PAD, D), f32)
    PA[...] = jnp.zeros((SEG, D), f32)

    cp_l.wait()
    HL[...] = _ln(xl[...].astype(f32).reshape(RPRE, D))

    def load_pair(hp, _):
        for c in w_copies(hp):
            c.wait()

        @pl.when(hp + 2 < NP)
        def _():
            for c in w_copies(hp + 2):
                c.start()

        wo_copy(hp).start()

        @pl.when(hp == NP - 1)
        def _():
            cp_b[0].start()
        slot = hp % NSLOT
        for a in range(3):
            PRE[hp, :, a * PW:(a + 1) * PW] = _dot(HL[...], stage[slot, a], NT)
            for kt in range(D // 128):
                t = stage[slot, a, :, kt * 128:(kt + 1) * 128].T
                wqkv[hp, kt * 64:(kt + 1) * 64, a * PW:(a + 1) * PW] = pltpu.bitcast(t, jnp.int32)
        X[pl.ds(pl.multiple_of(hp * XS * SEG, XS * SEG), XS * SEG), :] = (
            xb[pl.ds(hp * XS, XS)].astype(f32).reshape(XS * SEG, D))
        return 0
    jax.lax.fori_loop(0, NP, load_pair, 0)

    cp_m.wait()
    for hp in range(NP):
        wo_copy(hp).wait()
    cp_b[0].wait()
    for c in cp_b[1:]:
        c.start()

    lane64 = jax.lax.broadcasted_iota(jnp.int32, (L, 128), 1) < 64
    ri = jax.lax.broadcasted_iota(jnp.int32, (L, 2 * L), 0)
    ci = jax.lax.broadcasted_iota(jnp.int32, (L, 2 * L), 1)
    first = ci < L
    causal = (ri < M) | (ri >= jnp.where(first, ci, ci - L))

    def seg_rows(s, off=0):
        return pl.ds(pl.multiple_of(s * SEG + off, M), SEG)

    def b1_norm(s):
        y = _ln(X[seg_rows(s), :])
        Y[seg_rows(s), :] = y
        Z[...] = _ln(y)

    def b1_dot(c0=0, c1=D // 128):
        cols = slice(c0 * 128, c1 * 128)
        PA[:, cols] = _dot(Z[...], _w(w1_s[:, cols]))

    def b1_act(s):
        HB[seg_rows(s, PAD), :] = _gelu(PA[...])

    def a_step(s, mem, pre):
        rows = pl.ds(pl.multiple_of(s * SEG, SEG), SEG)
        nin = SIN if pre else SEG
        h = jnp.concatenate([mem, H[pl.ds(pl.multiple_of(s * SEG, SEG), nin), :]], axis=0)
        if pre:
            h = h.astype(bf16)
        sc, pr = {}, {}
        acc = [None]

        def st_proj(hp, a0, a1):
            cols = slice(a0 * PW, a1 * PW)
            qkv_s[hp, 0:M + nin, cols] = _dot(h, _w(wqkv[hp, :, cols]))

        def part(hp, a):
            v = qkv_s[hp, 0:M + nin, a * PW:(a + 1) * PW]
            if pre:
                v = jnp.concatenate(
                    [v, PRE[hp, pl.ds(pl.multiple_of(s * M, M), M), a * PW:(a + 1) * PW]], axis=0)
            return v

        def st_qk(hp):
            sc[hp] = _dot(part(hp, 0), _blockdiag(part(hp, 1), lane64), NT)

        def st_softmax(hp):
            v = jnp.where(causal, sc.pop(hp), -1e9 / SCALE)
            m0 = jnp.max(jnp.where(first, v, -jnp.inf), axis=1, keepdims=True)
            m1 = jnp.max(jnp.where(first, -jnp.inf, v), axis=1, keepdims=True)
            pr[hp] = jnp.exp2((v - jnp.where(first, m0, m1)) * (SCALE * LOG2E))

        def st_pv(hp):
            e = pr.pop(hp)
            pv = _dot(e, _blockdiag(part(hp, 2), lane64))
            i0 = 1.0 / jnp.sum(jnp.where(first, e, 0.0), axis=1, keepdims=True)
            i1 = 1.0 / jnp.sum(jnp.where(first, 0.0, e), axis=1, keepdims=True)
            o_s[:, hp * PW:(hp + 1) * PW] = jnp.concatenate(
                [pv[:, 0:128] * i0, pv[:, 128:256] * jnp.where(lane64, i0, i1), pv[:, 256:384] * i1],
                axis=1)

        def st_out(hp):
            t = _dot(o_s[:, hp * PW:(hp + 1) * PW], _w(wo_s[hp * DH:(hp + 1) * DH, :]))
            acc[0] = t if acc[0] is None else acc[0] + t

        nrows = seg_rows(jnp.minimum(s + 1, NSEG - 1))
        H[nrows, :] = _ln(X[nrows, :])
        b1_act(jnp.maximum(s - 2, 0))
        b1_norm(jnp.maximum(s - 1, 0))

        for i in range(NP + 4):
            if 0 <= i - 2 < NP:
                st_softmax(i - 2)
            if i < NP:
                st_proj(i, 0, 2)
            if i == NP:
                b1_dot(0, 2)
            if 0 <= i - 1 < NP:
                st_qk(i - 1)
            if 0 <= i - 3 < NP:
                st_pv(i - 3)
            if i < NP:
                st_proj(i, 2, 3)
            if 0 <= i - 4 < NP:
                st_out(i - 4)
        b1_dot(2, D // 128)
        X[rows, :] = X[rows, :] + acc[0][M:, :]
        return acc[0][:M, :]

    TH = TB // NH_B
    lane = jax.lax.broadcasted_iota(jnp.int32, (TH, 128), 1)

    def b_chunk(i, layer, tail=False):
        mo = (lambda v, m: v) if isinstance(i, int) else pl.multiple_of
        r = pl.ds(mo(i * TB, TB), TB)
        rows = [pl.ds(mo(i * TB + u * TH, TH), TH) for u in range(NH_B)]

        def mixed(u):
            win = HB[pl.ds(mo(i * TB + u * TH, TH), TH + 2 * PAD), :]

            def sh(ct, d):
                return win[PAD + d:PAD + d + TH, ct * 128:(ct + 1) * 128]
            return jnp.concatenate([
                sh(0, -1),
                jnp.where(lane < 32, sh(1, -1), sh(1, 1)),
                jnp.where(lane < 64, sh(2, 1), sh(2, -2)),
                jnp.where(lane < 96, sh(3, -2), sh(3, 2)),
                sh(4, 2)], axis=1)

        if tail:
            b1_act(NSEG - 2)
            b1_norm(NSEG - 1)
        x1 = [Y[rows[u], :] + _dot(mixed(u), _w(w2_s[...])) for u in range(NH_B)]
        if tail:
            b1_dot()
            b1_act(NSEG - 1)
        g = [_gelu(_dot(_ln(x1[u]), _w(w3_s[...]))) for u in range(NH_B)]
        for u in range(NH_B):
            xn = X[rows[u], :] + (x1[u] + _dot(g[u], _w(w4_s[...])))
            X[rows[u], :] = xn
            ob[rows[u], :] = xn.astype(bf16)

        @pl.when(layer == 1)
        def _():
            pltpu.make_async_copy(ob.at[r, :], out_hbm.at[r, :], sem_o.at[i]).start()
        return layer

    def layer_body(layer, _):
        H[0:SEG, :] = _ln(X[0:SEG, :])

        def a_steps(j, mem, pre):
            for u in range(UNR):
                mem = a_step(j * UNR + u, mem, pre)
            return mem
        npre = jnp.where(layer == 0, NPRE // UNR, 0)
        mem = jax.lax.fori_loop(0, npre, functools.partial(a_steps, pre=True),
                                memb[0:M, :].astype(f32))
        jax.lax.fori_loop(npre, NSEG // UNR, functools.partial(a_steps, pre=False), mem)

        @pl.when(layer == 0)
        def _():
            for c in cp_b[1:]:
                c.wait()
        b_chunk(0, layer, tail=True)
        jax.lax.fori_loop(1, NB, b_chunk, layer)
        return 0

    jax.lax.fori_loop(0, 2, layer_body, 0)

    for i in range(NB):
        pltpu.make_async_copy(ob.at[pl.ds(i * TB, TB), :], out_hbm.at[pl.ds(i * TB, TB), :],
                              sem_o.at[i]).wait()


def pallas_interleave_layers__memory_aug_recurrent_mem_tr__mixer_s_mlp__prompt_kernel(
    A_x: jax.Array,
    A_mem0: jax.Array,
    A_Wq: jax.Array,
    A_Wk: jax.Array,
    A_Wv: jax.Array,
    A_Wo: jax.Array,
    A_seg_len,
    B_x: jax.Array,
    B_w1: jax.Array,
    B_w2: jax.Array,
    B_w3: jax.Array,
    B_w4: jax.Array,
):
    del A_seg_len, B_x

    def wt(w):
        return jnp.transpose(w, (1, 2, 0)).reshape(NH * DH, D)

    any_spec = pl.BlockSpec(memory_space=pl.ANY)
    out = pl.pallas_call(
        _kernel,
        out_shape=jax.ShapeDtypeStruct((S, D), bf16),
        in_specs=[any_spec] * 10,
        out_specs=any_spec,
        scratch_shapes=[
            pltpu.VMEM((NSEG, SEG, D), bf16),
            pltpu.VMEM((NPRE, M, D), bf16),
            pltpu.VMEM((64, D), bf16),
            pltpu.VMEM((NSLOT, 3, PW, D), bf16),
            pltpu.VMEM((NP, D // 2, 3 * PW), jnp.int32),
            pltpu.VMEM((NH * DH // 2, D), jnp.int32),
            pltpu.VMEM((D // 2, D), jnp.int32),
            pltpu.VMEM((D // 2, D), jnp.int32),
            pltpu.VMEM((D // 2, F), jnp.int32),
            pltpu.VMEM((F // 2, D), jnp.int32),
            pltpu.VMEM((S, D), f32),
            pltpu.VMEM((S, D), f32),
            pltpu.VMEM((S, D), f32),
            pltpu.VMEM((S + 32, D), f32),
            pltpu.VMEM((RPRE, D), f32),
            pltpu.VMEM((NP, RPRE, 3 * PW), f32),
            pltpu.VMEM((NP, L, 3 * PW), f32),
            pltpu.VMEM((L, NH * DH), f32),
            pltpu.VMEM((SEG, D), f32),
            pltpu.VMEM((SEG, D), f32),
            pltpu.VMEM((S, D), bf16),
            pltpu.SemaphoreType.DMA((2,)),
            pltpu.SemaphoreType.DMA((NSLOT,)),
            pltpu.SemaphoreType.DMA((5,)),
            pltpu.SemaphoreType.DMA((NB,)),
        ],
        compiler_params=pltpu.CompilerParams(vmem_limit_bytes=120 * 1024 * 1024),
    )(A_x.reshape(NSEG, SEG, D), A_mem0.reshape(M, D), wt(A_Wq), wt(A_Wk), wt(A_Wv),
      A_Wo.reshape(NH * DH, D), B_w1, B_w2, B_w3, B_w4)
    return out.reshape(1, S, D)
```
